```python
import jax
import jax.numpy as jnp

def _softmax(x, axis=-1):
    return jax.nn.softmax(x, axis=axis)
def _gelu(x):
    return jax.nn.gelu(x, approximate=True)
def _silu(x):
    return jax.nn.silu(x)
def _sigmoid(x):
    return jax.nn.sigmoid(x)
def _layernorm(x, axis=-1, eps=1e-5):
    m = jnp.mean(x, axis=axis, keepdims=True)
    v = jnp.var(x, axis=axis, keepdims=True)
    return (x - m) / jnp.sqrt(v + eps)
def _scatter_add(tgt, idx, src, axis=0):
    return tgt.at[idx].add(src)
def _segment_sum(src, seg, n):
    return jax.ops.segment_sum(src, seg, n)
class _Rng:
    def __init__(self, key):
        self._k = key
    def _next(self):
        self._k, sub = jax.random.split(self._k)
        return sub
    def normal(self, shape):
        return jax.random.normal(self._next(), shape, dtype=jnp.bfloat16)
    def randint(self, lo, hi, shape):
        return jax.random.randint(self._next(), shape, lo, hi, dtype=jnp.int32)
    def uniform(self, shape, lo=0.0, hi=1.0):
        return jax.random.uniform(self._next(), shape, jnp.bfloat16, lo, hi)
    def permutation(self, n):
        return jax.random.permutation(self._next(), n)


kernel_name = 'gated_mix__sliding_local_dilated__glu_gated_reglu__prompt'

def setup_inputs():
    _rng = _Rng(jax.random.key(int.from_bytes(__import__("os").urandom(4), "little")))
    _w = (lambda a: (lambda t: t.astype(jnp.bfloat16) if jnp.issubdtype(t.dtype, jnp.floating) else t)(jnp.asarray(a)))
    def _A_setup():
        B, S, D = 1, 2048, 1024
        return {
            "x": _w((lambda *s: _rng.normal(s) * 0.05)(B, S, D)),
            "wqkv": _w((lambda *s: _rng.normal(s) * 0.05)(D, 3 * D)),
            "wo": _w((lambda *s: _rng.normal(s) * 0.05)(D, D)),
        }
    _A_in = _A_setup()

    def _B_setup():
        B, S, D, F = 1, 2048, 1024, 3584
        return {
            "x": _w((lambda *s: _rng.normal(s) * 0.05)(B, S, D)),
            "W_gate": _w((lambda *s: _rng.normal(s) * 0.05)(D, F) * (2.0 / D) ** 0.5),
            "W_up": _w((lambda *s: _rng.normal(s) * 0.05)(D, F) * (2.0 / D) ** 0.5),
            "W_down": _w((lambda *s: _rng.normal(s) * 0.05)(F, D) * (1.0 / F) ** 0.5),
        }
    _B_in = _B_setup()

    return {
        "A_x": _A_in["x"],
        "A_wqkv": _A_in["wqkv"],
        "A_wo": _A_in["wo"],
        "B_x": _B_in["x"],
        "B_W_gate": _B_in["W_gate"],
        "B_W_up": _B_in["W_up"],
        "B_W_down": _B_in["W_down"],
        "gate_w": _w((lambda *s: _rng.normal(s) * 0.05)(1024)),
    }

def reference(A_x, A_wqkv, A_wo, B_x, B_W_gate, B_W_up, B_W_down, gate_w):
    def _A_ref(x, wqkv, wo):
        B, S, D = x.shape
        H = 32; Dh = D // H
        W, dil = 8, 2
        qkv = (lambda x, *d: x.transpose(*d))((x @ wqkv).reshape(B, S, 3, H, Dh), 2, 0, 3, 1, 4)
        q, k, v = qkv[0], qkv[1], qkv[2]
        scale = Dh ** -0.5
        pos = jnp.arange(S)
        off = jnp.arange(W) * dil
        idx = pos[:, None] - off[None, :]
        mask = idx >= 0
        idx_c = jnp.where(mask, idx, 0).reshape(-1)
        kg = k[:, :, idx_c, :].reshape(B, H, S, W, Dh)
        vg = v[:, :, idx_c, :].reshape(B, H, S, W, Dh)
        logits = jnp.einsum("bhsd,bhswd->bhsw", q, kg) * scale
        logits = jnp.where(mask[None, None, :, :], logits, -1e9)
        attn = _softmax(logits, axis=-1)
        o = jnp.einsum("bhsw,bhswd->bhsd", attn, vg)
        return (lambda x, *d: x.transpose(*d))(o, 0, 2, 1, 3).reshape(B, S, D) @ wo

    def _B_ref(x, W_gate, W_up, W_down):
        gate = jnp.einsum("bsd,df->bsf", x, W_gate)
        up = jnp.einsum("bsd,df->bsf", x, W_up)
        gate = gate * (lambda x, dt: x.astype(dt))(gate > 0, gate.dtype)
        h = gate * up
        return jnp.einsum("bsf,fd->bsd", h, W_down)

    x = A_x
    g = _sigmoid((x * gate_w).sum(-1, keepdims=True))
    a = _A_ref(x, A_wqkv, A_wo)
    b = _B_ref(x, B_W_gate, B_W_up, B_W_down)
    return g * a + (1 - g) * b
```

```python
import jax
import jax.numpy as jnp
from jax import lax
import jax.experimental.pallas as pl
import jax.experimental.pallas.tpu as pltpu

H = 32
WIN = 8
DIL = 2
HALO = 16
LANES = 128
NEG = -1e9

R1 = 512
FC1 = 256
FC2 = 512
NIT = 8
PITCH = 17

TOK_PAIRS = ((0, 2), (4, 6), (8, 12))

F32 = jnp.float32
BF16 = jnp.bfloat16
U32 = jnp.uint32


def _dot(a, b):
    return jnp.dot(a, b, preferred_element_type=F32)


def _dot_nt(a, b):
    return lax.dot_general(a, b, (((1,), (1,)), ((), ())), preferred_element_type=F32)


def _kernel(x_hbm, wqkv_hbm, wo_hbm, wg_hbm, wu_hbm, wd_hbm, gw_hbm, out_hbm,
            x_v, wqkv_v, wo_v, wg_v, wu_v, wd_v, gw_v,
            wt_v, wop_v, tmp_v, b_v, q_v, k_v, v_v, o_v, out_v,
            sem_in, sem_out, *, S, D, F):
    NCH = D // LANES
    DH = D // H
    scale = DH ** -0.5
    n1 = F // FC1
    n2 = F // FC2
    MF = (S - R1) // NIT
    MA = S // NIT
    NU = 3 * NCH

    sidx = [0]

    def _next():
        sidx[0] += 1
        return sidx[0] - 1

    s_x0 = _next(); s_gw = _next(); s_xr = _next()
    s_w = sidx[0]; sidx[0] += 3 * n1
    s_u = sidx[0]; sidx[0] += NU
    s_o = sidx[0]; sidx[0] += NCH

    def cp_x0():
        return pltpu.make_async_copy(x_hbm.at[0, pl.ds(0, R1), :], x_v.at[pl.ds(0, R1), :], sem_in.at[s_x0])

    def cp_xr():
        return pltpu.make_async_copy(x_hbm.at[0, pl.ds(R1, S - R1), :], x_v.at[pl.ds(R1, S - R1), :],
                                     sem_in.at[s_xr])

    def cp_gw():
        return pltpu.make_async_copy(gw_hbm, gw_v, sem_in.at[s_gw])

    def _off(c, n):
        return c * n if isinstance(c, int) else pl.multiple_of(c * n, n)

    def cp_g(c):
        sl = pl.ds(_off(c, FC1), FC1)
        return pltpu.make_async_copy(wg_hbm.at[:, sl], wg_v.at[:, sl], sem_in.at[s_w + 3 * c])

    def cp_u(c):
        sl = pl.ds(_off(c, FC1), FC1)
        return pltpu.make_async_copy(wu_hbm.at[:, sl], wu_v.at[:, sl], sem_in.at[s_w + 3 * c + 1])

    def cp_d(c):
        sl = pl.ds(_off(c, FC1), FC1)
        return pltpu.make_async_copy(wd_hbm.at[sl, :], wd_v.at[sl, :], sem_in.at[s_w + 3 * c + 2])

    def cp_wq(u):
        sec, kb = u // NCH, u % NCH
        return pltpu.make_async_copy(
            wqkv_hbm.at[pl.ds(_off(kb, LANES), LANES), pl.ds(_off(sec, D), D)],
            wqkv_v.at[u], sem_in.at[s_u + u])

    def cp_wo(c):
        return pltpu.make_async_copy(wo_hbm.at[:, pl.ds(_off(c, LANES), LANES)], wo_v.at[c],
                                     sem_in.at[s_o + c])

    def cp_out(i):
        sl = pl.ds(_off(i, MA), MA)
        return pltpu.make_async_copy(out_v.at[sl, :], out_hbm.at[0, sl, :], sem_out.at[i])

    cp_x0().start()
    for c in range(n1):
        cp_g(c).start(); cp_u(c).start(); cp_d(c).start()
        if c == 0:
            cp_gw().start()
        if c >= 1:
            for u in (2 * (c - 1), 2 * (c - 1) + 1):
                if u < NU:
                    cp_wq(u).start()
            if c - 1 < NCH:
                cp_wo(c - 1).start()
    cp_xr().start()

    def ffn_chunk(xv, off, fc):
        g = _dot(xv, wg_v[:, pl.ds(off, fc)])
        u = _dot(xv, wu_v[:, pl.ds(off, fc)])
        h = (jnp.maximum(g, 0.0) * u).astype(BF16)
        r = _dot(h, wd_v[pl.ds(off, fc), :])
        toks = [m[0:8, t * LANES:(t + 1) * LANES] for m in (g, u, r) for t in range(m.shape[1] // LANES)]
        return r, toks

    def permute_rows(slot, u32, dst, row0, col):
        for g in range(2 * H):
            tmp_v[slot, pl.ds((g // 2) * PITCH + (g % 2) * 8, 8), :] = u32[g * 8:(g + 1) * 8, :]
        for j in range(NCH):
            for e in range(2):
                base = row0 + (2 * j + e) * H
                if not isinstance(base, int):
                    base = pl.multiple_of(base, H)
                dst[pl.ds(base, H), col] = tmp_v[slot, pl.ds(8 * e + j, H, stride=PITCH), :]

    def prep_wq(slot, u):
        sec, kb = u // NCH, u % NCH
        u32 = pltpu.bitcast(wqkv_v[u].T, U32)
        permute_rows(slot, u32, wt_v, _off(sec, D // 2), pl.ds(_off(kb, LANES), LANES))
        tok = u32[0:8, :]
        for t in range(1, NCH):
            tok = tok | u32[t * 64:t * 64 + 8, :]
        return tok

    def prep_wo(slot, c, never, tok):
        u32 = pltpu.bitcast(wo_v[c], U32)
        u32 = jnp.concatenate(
            [jnp.where(never, tok, u32[g * 8:(g + 1) * 8, :]) for g in range(2 * H)], axis=0)
        permute_rows(slot, u32, wop_v, 0, pl.ds(_off(c, LANES), LANES))

    def qkv(xa):
        for sec, dst, r0 in ((1, k_v, HALO), (0, q_v, 0), (2, v_v, HALO)):
            res = _dot_nt(xa, pltpu.bitcast(wt_v[sec * (D // 2):(sec + 1) * (D // 2), :], BF16))
            for j in range(NCH):
                dst[j, r0:r0 + MA, :] = res[:, j * LANES:(j + 1) * LANES]

    lane8 = lax.broadcasted_iota(jnp.int32, (8, LANES), 1)
    odd = (lane8 & 1) == 1
    row8 = lax.broadcasted_iota(jnp.int32, (8, LANES), 0)

    def attn8(r, row0, tok):
        sc = jnp.where(row8 + row0 < 0, tok, scale)
        q = [q_v[j, r:r + 8, :] * sc for j in range(NCH)]
        logits = []
        for w in range(WIN):
            lo = HALO + r - DIL * w
            s = q[0] * k_v[0, lo:lo + 8, :]
            for j in range(1, NCH):
                s = s + q[j] * k_v[j, lo:lo + 8, :]
            s = s + pltpu.roll(s, 64, 1)
            s = s + jnp.where(odd, pltpu.roll(s, 1, 1), pltpu.roll(s, LANES - 1, 1))
            if r - DIL * w < 0:
                s = jnp.where(row8 + (row0 + r - DIL * w) >= 0, s, NEG)
            logits.append(s)
        m = logits[0]
        for w in range(1, WIN):
            m = jnp.maximum(m, logits[w])
        p = [jnp.exp(l - m) for l in logits]
        den = p[0]
        for w in range(1, WIN):
            den = den + p[w]
        inv = 1.0 / den
        p = [pw * inv for pw in p]
        outs = []
        for j in range(NCH):
            acc = p[0] * v_v[j, HALO + r:HALO + r + 8, :]
            for w in range(1, WIN):
                lo = HALO + r - DIL * w
                acc = acc + p[w] * v_v[j, lo:lo + 8, :]
            outs.append(acc)
        return outs

    def attn16(r, row0, tok_a, tok_b):
        a = attn8(r, row0, tok_a)
        b = attn8(r + 8, row0, tok_b)
        for j in range(NCH):
            o_v[r // 2:r // 2 + 8, j * LANES:(j + 1) * LANES] = pltpu.bitcast(
                jnp.concatenate([a[j], b[j]], axis=0).astype(BF16), U32)

    cp_x0().wait()
    cp_g(0).wait()
    xv = x_v[0:R1, :]
    g = _dot(xv, wg_v[:, 0:FC1])
    cp_u(0).wait()
    u = _dot(xv, wu_v[:, 0:FC1])
    h = (jnp.maximum(g, 0.0) * u).astype(BF16)
    cp_d(0).wait()
    b_v[0:R1, :] = _dot(h, wd_v[0:FC1, :])

    def p1_body(c, carry):
        cp_g(c).wait(); cp_u(c).wait(); cp_d(c).wait()

        @pl.when(2 * (c - 1) < NU)
        def _():
            cp_wq(2 * (c - 1)).wait()
            cp_wq(2 * (c - 1) + 1).wait()

        @pl.when(c - 1 < NCH)
        def _():
            cp_wo(c - 1).wait()

        u0 = jnp.minimum(2 * (c - 1), NU - 2)
        off = _off(c, FC1)
        xv = x_v[0:R1, :]
        never = row8 + c < 0
        g = _dot(xv, wg_v[:, pl.ds(off, FC1)])
        u = _dot(xv, wu_v[:, pl.ds(off, FC1)])
        tok = prep_wq(0, u0) | prep_wq(1, u0 + 1)
        prep_wo(2, jnp.minimum(c - 1, NCH - 1), never, pltpu.bitcast(g[0:8, 0:LANES], U32))
        zero = jnp.where(never, pltpu.bitcast(tok, F32), 0.0)
        g0 = jnp.concatenate([jnp.maximum(g[0:8, 0:LANES], zero), g[0:8, LANES:]], axis=1)
        g = jnp.concatenate([g0, g[8:, :]], axis=0)
        h = (jnp.maximum(g, 0.0) * u).astype(BF16)
        b_v[0:R1, :] += _dot(h, wd_v[pl.ds(off, FC1), :])
        return carry

    lax.fori_loop(1, n1, p1_body, 0)

    cp_gw().wait()
    cp_xr().wait()
    k_v[:, MA:MA + HALO, :] = jnp.zeros((NCH, HALO, LANES), F32)
    v_v[:, MA:MA + HALO, :] = jnp.zeros((NCH, HALO, LANES), F32)

    ngrp = MA // 16

    def p2_body(i, carry):
        ra = pl.multiple_of(i * MA, MA)
        rf = pl.multiple_of(R1 + i * MF, 16)
        k_v[:, 0:HALO, :] = k_v[:, MA:MA + HALO, :]
        v_v[:, 0:HALO, :] = v_v[:, MA:MA + HALO, :]
        qkv(x_v[pl.ds(ra, MA), :])
        gi = 0
        for c in range(n2):
            r, toks = ffn_chunk(x_v[pl.ds(rf, MF), :], c * FC2, FC2)
            if c == 0:
                b_v[pl.ds(rf, MF), :] = r
            else:
                b_v[pl.ds(rf, MF), :] += r
            for ta, tb in TOK_PAIRS:
                if gi < ngrp:
                    attn16(gi * 16, ra, toks[ta], toks[tb])
                    gi += 1
        gw = gw_v[...].astype(F32)
        z = jnp.sum(x_v[pl.ds(ra, MA), :].astype(F32) * gw, axis=-1, keepdims=True)
        gate = jax.nn.sigmoid(z)
        a = _dot(pltpu.bitcast(o_v[...], BF16), pltpu.bitcast(wop_v[...], BF16))
        b = b_v[pl.ds(ra, MA), :]
        out_v[pl.ds(ra, MA), :] = (gate * a + (1.0 - gate) * b).astype(BF16)
        cp_out(i).start()
        return carry

    lax.fori_loop(0, NIT, p2_body, 0)
    for i in range(NIT):
        cp_out(i).wait()


@jax.jit
def pallas_gated_mix__sliding_local_dilated__glu_gated_reglu__prompt_kernel(
    A_x: jax.Array,
    A_wqkv: jax.Array,
    A_wo: jax.Array,
    B_x: jax.Array,
    B_W_gate: jax.Array,
    B_W_up: jax.Array,
    B_W_down: jax.Array,
    gate_w: jax.Array,
):
    B, S, D = A_x.shape
    assert B == 1
    F = B_W_gate.shape[1]
    NCH = D // LANES
    MA = S // NIT
    n_in = 3 + 3 * (F // FC1) + 3 * NCH + NCH

    def kernel(*refs):
        _kernel(*refs, S=S, D=D, F=F)

    any_spec = pl.BlockSpec(memory_space=pl.ANY)
    return pl.pallas_call(
        kernel,
        in_specs=[any_spec] * 7,
        out_specs=any_spec,
        out_shape=jax.ShapeDtypeStruct((B, S, D), A_x.dtype),
        scratch_shapes=[
            pltpu.VMEM((S, D), BF16),
            pltpu.VMEM((3 * NCH, LANES, D), BF16),
            pltpu.VMEM((NCH, D, LANES), BF16),
            pltpu.VMEM((D, F), BF16),
            pltpu.VMEM((D, F), BF16),
            pltpu.VMEM((F, D), BF16),
            pltpu.VMEM((1, D), BF16),
            pltpu.VMEM((3 * D // 2, D), U32),
            pltpu.VMEM((D // 2, D), U32),
            pltpu.VMEM((3, H * PITCH + 7, LANES), jnp.uint32),
            pltpu.VMEM((S, D), F32),
            pltpu.VMEM((NCH, MA, LANES), F32),
            pltpu.VMEM((NCH, HALO + MA, LANES), F32),
            pltpu.VMEM((NCH, HALO + MA, LANES), F32),
            pltpu.VMEM((MA // 2, D), U32),
            pltpu.VMEM((S, D), BF16),
            pltpu.SemaphoreType.DMA((n_in,)),
            pltpu.SemaphoreType.DMA((NIT,)),
        ],
        compiler_params=pltpu.CompilerParams(
            vmem_limit_bytes=100 * 1024 * 1024,
            disable_semaphore_checks=True,
            disable_bounds_checks=True,
        ),
    )(A_x, A_wqkv, A_wo, B_W_gate, B_W_up, B_W_down, gate_w.reshape(1, D))
```

```python
import jax
import jax.numpy as jnp
from jax import lax
import jax.experimental.pallas as pl
import jax.experimental.pallas.tpu as pltpu

H = 32
WIN = 8
DIL = 2
HALO = 16
LANES = 128
NEG = -1e9

R1 = 512
FC1 = 512
FC2 = 512
NIT = 8
PITCH = 17

TOKS = ((0, 1, 3), (4, 5, 7), (8, 10, 14))
UQ = 5
UO = 2
NAUX = 4
P1_LAG = 2
TMP_ROWS = 552
KV_PAD = 0

PEEL_COPIES = (("x", 0, 256), ("g", 0, 256), ("x", 256, 512), ("u", 0, 256),
               ("g", 256, 512), ("u", 256, 512), ("d", 0, 512))
PEEL_STEPS = (
    ((0, 1), (("g", 0, 256, 0, 256),)),
    ((2,), (("g", 256, 512, 0, 256),)),
    ((3,), (("u", 0, 512, 0, 256), ("h", 0, 512, 0, 256))),
    ((4, 5), (("g", 0, 512, 256, 512), ("u", 0, 512, 256, 512), ("h", 0, 512, 256, 512))),
    ((6,), (("d", 0, 512, 0, 512),)),
)

F32 = jnp.float32
BF16 = jnp.bfloat16
U32 = jnp.uint32


def _dot(a, b):
    return jnp.dot(a, b, preferred_element_type=F32)


def _dot_nt(a, b):
    return lax.dot_general(a, b, (((1,), (1,)), ((), ())), preferred_element_type=F32)


def _kernel(x_hbm, wqkv_hbm, wo_hbm, wg_hbm, wu_hbm, wd_hbm, gw_hbm, out_hbm,
            x_v, wqkv_v, wo_v, wg_v, wu_v, wd_v, gw_v,
            wt_v, wop_v, tmp_v, b_v, q_v, k_v, v_v, o_v, og_v, out_v,
            sem_in, sem_out, *, S, D, F):
    NCH = D // LANES
    DH = D // H
    scale = DH ** -0.5
    n1 = F // FC1
    n2 = F // FC2
    MF = (S - R1) // NIT
    MA = S // NIT
    NU = 3 * NCH
    Q0 = 2 * UQ
    O0 = 2 * UO
    assert UQ * (n1 - 1) + UQ - 1 - Q0 >= NU - 1 and UO * (n1 - 1) + UO - 1 - O0 >= NCH - 1

    x_h = x_hbm.at[0].bitcast(U32)
    out_h = out_hbm.at[0].bitcast(U32)
    wqkv_h, wo_h, wg_h, wu_h, wd_h = (r.bitcast(U32) for r in (wqkv_hbm, wo_hbm, wg_hbm, wu_hbm, wd_hbm))

    def _off(c, n):
        return c * n if isinstance(c, int) else pl.multiple_of(c * n, n)

    def rows(start, n):
        if isinstance(start, int):
            return pl.ds(start // 2, n // 2)
        return pl.ds(pl.multiple_of(start // 2, 8), n // 2)

    def bf(v):
        return pltpu.bitcast(v, BF16)

    s_p = 0
    s_gw = len(PEEL_COPIES)
    s_xr = s_gw + 1
    s_w = s_xr + 1 - 3
    s_u = s_w + 3 * n1
    s_o = s_u + NAUX

    def cp_peel(n):
        kind, lo, hi = PEEL_COPIES[n]
        if kind == "x":
            sl = rows(lo, hi - lo)
            return pltpu.make_async_copy(x_h.at[sl, :], x_v.at[sl, :], sem_in.at[s_p + n])
        if kind == "d":
            sl = rows(lo, hi - lo)
            return pltpu.make_async_copy(wd_h.at[sl, :], wd_v.at[sl, :], sem_in.at[s_p + n])
        src, dst = (wg_h, wg_v) if kind == "g" else (wu_h, wu_v)
        sl = pl.ds(lo, hi - lo)
        return pltpu.make_async_copy(src.at[:, sl], dst.at[:, sl], sem_in.at[s_p + n])

    def cp_xr():
        sl = rows(R1, S - R1)
        return pltpu.make_async_copy(x_h.at[sl, :], x_v.at[sl, :], sem_in.at[s_xr])

    def cp_gw():
        return pltpu.make_async_copy(gw_hbm, gw_v, sem_in.at[s_gw])

    def cp_g(c):
        sl = pl.ds(_off(c, FC1), FC1)
        return pltpu.make_async_copy(wg_h.at[:, sl], wg_v.at[:, sl], sem_in.at[s_w + 3 * c])

    def cp_u(c):
        sl = pl.ds(_off(c, FC1), FC1)
        return pltpu.make_async_copy(wu_h.at[:, sl], wu_v.at[:, sl], sem_in.at[s_w + 3 * c + 1])

    def cp_d(c):
        sl = pl.ds(_off(c, FC1 // 2), FC1 // 2)
        return pltpu.make_async_copy(wd_h.at[sl, :], wd_v.at[sl, :], sem_in.at[s_w + 3 * c + 2])

    def cp_wq(t):
        sl = pl.ds(_off(t, D // NAUX // 2), D // NAUX // 2)
        return pltpu.make_async_copy(wqkv_h.at[sl, :], wqkv_v.at[sl, :], sem_in.at[s_u + t])

    def cp_wo(t):
        sl = pl.ds(_off(t, D // NAUX), D // NAUX)
        return pltpu.make_async_copy(wo_h.at[:, sl], wo_v.at[:, sl], sem_in.at[s_o + t])

    def cp_out(i):
        sl = pl.ds(_off(i, MA // 2), MA // 2)
        return pltpu.make_async_copy(out_v.at[sl, :], out_h.at[sl, :], sem_out.at[i])

    for n in range(len(PEEL_COPIES)):
        cp_peel(n).start()
    for c in range(1, n1):
        cp_g(c).start(); cp_u(c).start(); cp_d(c).start()
        if 0 <= c - 2 < NAUX:
            cp_wq(c - 2).start(); cp_wo(c - 2).start()
    cp_gw().start()
    cp_xr().start()

    lane8 = lax.broadcasted_iota(jnp.int32, (8, LANES), 1)
    odd = (lane8 & 1) == 1
    row8 = lax.broadcasted_iota(jnp.int32, (8, LANES), 0)

    def ffn_chunk(xv, off, fc):
        g = _dot(xv, bf(wg_v[:, pl.ds(off, fc)]))
        u = _dot(xv, bf(wu_v[:, pl.ds(off, fc)]))
        h = (jnp.maximum(g, 0.0) * u).astype(BF16)
        r = _dot(h, bf(wd_v[rows(off, fc), :]))
        toks = [m[0:8, t * LANES:(t + 1) * LANES] for m in (g, u, r) for t in range(m.shape[1] // LANES)]
        return r, toks

    def permute_rows(slot, u32, dst, row0, col):
        for g in range(2 * H):
            tmp_v[slot, pl.ds((g // 2) * PITCH + (g % 2) * 8, 8), :] = u32[g * 8:(g + 1) * 8, :]
        for j in range(NCH):
            for e in range(2):
                base = row0 + (2 * j + e) * H
                if not isinstance(base, int):
                    base = pl.multiple_of(base, H)
                dst[col, pl.ds(base, H), :] = tmp_v[slot, pl.ds(8 * e + j, H, stride=PITCH), :]

    def after(never, tok, u32):
        return jnp.concatenate(
            [jnp.concatenate([jnp.where(never, tok, u32[r:r + 8, c:c + LANES])
                              for c in range(0, u32.shape[1], LANES)], axis=1)
             for r in range(0, u32.shape[0], 8)], axis=0)

    def prep_wq(slot, u, never, tok):
        kb, sec = u // 3, u % 3
        raw = wqkv_v[pl.ds(_off(kb, LANES // 2), LANES // 2), pl.ds(_off(sec, D), D)]
        u32 = pltpu.bitcast(bf(after(never, tok, raw)).T, U32)
        permute_rows(slot, u32, wt_v, _off(sec, D // 2), kb)
        tok = u32[56:64, :]
        for t in range(1, NCH):
            tok = tok | u32[t * 64 + 56:t * 64 + 64, :]
        return tok

    def prep_wo(slot, c, never, toks):
        n = D // 2 // len(toks)
        col = pl.ds(_off(c, LANES), LANES)
        u32 = jnp.concatenate([after(never, tok, wo_v[i * n:(i + 1) * n, col]) for i, tok in enumerate(toks)],
                              axis=0)
        permute_rows(slot, u32, wop_v, 0, c)

    def qkv(xa):
        for sec, dst, r0 in ((1, k_v, HALO), (0, q_v, 0), (2, v_v, HALO)):
            w = jnp.concatenate([wt_v[kb, sec * (D // 2):(sec + 1) * (D // 2), :] for kb in range(NCH)], axis=1)
            res = _dot_nt(xa, bf(w))
            for j in range(NCH):
                dst[j, r0:r0 + MA, :] = res[:, j * LANES:(j + 1) * LANES]

    def attn8(r, row0, never, tok, gate):
        sc = jnp.where(never, tok, scale)
        q = [q_v[j, r:r + 8, :] * sc for j in range(NCH)]
        logits = []
        for w in range(WIN):
            lo = HALO + r - DIL * w
            s = q[0] * k_v[0, lo:lo + 8, :]
            for j in range(1, NCH):
                s = s + q[j] * k_v[j, lo:lo + 8, :]
            s = s + pltpu.roll(s, 64, 1)
            s = s + jnp.where(odd, pltpu.roll(s, 1, 1), pltpu.roll(s, LANES - 1, 1))
            if r - DIL * w < 0:
                s = jnp.where(row8 + (row0 + r - DIL * w) >= 0, s, NEG)
            logits.append(s)
        m = logits[0]
        for w in range(1, WIN):
            m = jnp.maximum(m, logits[w])
        p = [jnp.exp(l - m) for l in logits]
        den = p[0]
        for w in range(1, WIN):
            den = den + p[w]
        inv = pl.reciprocal(den, approx=True)
        inv = inv * (2.0 - den * inv) * gate
        p = [pw * inv for pw in p]
        outs = []
        for j in range(NCH):
            acc = p[0] * v_v[j, HALO + r:HALO + r + 8, :]
            for w in range(1, WIN):
                lo = HALO + r - DIL * w
                acc = acc + p[w] * v_v[j, lo:lo + 8, :]
            outs.append(acc)
        return outs

    def attn16(r, row0, tok_g, tok_a, tok_b):
        never = row8 + row0 < 0
        xg = bf(after(never, pltpu.bitcast(tok_g, U32), x_v[rows(row0 + r, 16), :])).astype(F32)
        z = jnp.sum(xg * gw_v[...].astype(F32).reshape(1, D), axis=-1, keepdims=True)
        th = 0.5 * jnp.tanh(jnp.broadcast_to(0.5 * z, (16, LANES)))
        gate = 0.5 + th
        og_v[r:r + 16, :] = 0.5 - th
        a = attn8(r, row0, never, tok_a, gate[0:8])
        b = attn8(r + 8, row0, never, tok_b, gate[8:16])
        for j in range(NCH):
            o_v[r // 2:r // 2 + 8, j * LANES:(j + 1) * LANES] = pltpu.bitcast(
                jnp.concatenate([a[j], b[j]], axis=0).astype(BF16), U32)

    k_v[:, MA:MA + HALO, :] = jnp.zeros((NCH, HALO, LANES), F32)
    v_v[:, MA:MA + HALO, :] = jnp.zeros((NCH, HALO, LANES), F32)
    wqkv_v[D // 2:, 0:D] = jnp.zeros((LANES // 2, D), U32)
    wo_v[:, D:] = jnp.zeros((D // 2, LANES), U32)

    parts = {}
    for waits, work in PEEL_STEPS:
        for n in waits:
            cp_peel(n).wait()
        for kind, r0, r1, c0, c1 in work:
            if kind in "gu":
                w_v = wg_v if kind == "g" else wu_v
                parts[kind, r0, c0] = (r1, c1, _dot(bf(x_v[rows(r0, r1 - r0), :]), bf(w_v[:, c0:c1])))
            elif kind == "h":
                def gather(kd):
                    cols = []
                    for cc in sorted({k[2] for k in parts if k[0] == kd and c0 <= k[2] < c1}):
                        rs = sorted(k[1] for k in parts if k[0] == kd and k[2] == cc)
                        cols.append(jnp.concatenate([parts[kd, r, cc][2] for r in rs], axis=0))
                    return jnp.concatenate(cols, axis=1)
                parts["h", 0, c0] = (r1, c1, (jnp.maximum(gather("g"), 0.0) * gather("u")).astype(BF16))
            else:
                h = jnp.concatenate([parts[k][2] for k in sorted(parts) if k[0] == "h" and c0 <= k[2] < c1], axis=1)
                r = _dot(h, bf(wd_v[rows(c0, c1 - c0), :]))
                if c0 == 0:
                    b_v[0:R1, :] = r
                else:
                    b_v[0:R1, :] += r

    def p1_body(c, carry):
        uq = [UQ * c + t - Q0 for t in range(UQ)]
        uo = [UO * c + t - O0 for t in range(UO)]
        uq = [jnp.where(jnp.logical_and(u >= 0, u < NU), u, NU) for u in uq]
        uo = [jnp.where(jnp.logical_and(u >= 0, u < NCH), u, NCH) for u in uo]
        aux = jnp.logical_and(c >= 2, c < 2 + NAUX)
        ta = jnp.clip(c - 2, 0, NAUX - 1)
        last = c == n1 - 1
        waits = [(aux, cp_wq(ta)), (aux, cp_wo(ta)), (last, cp_gw()), (last, cp_xr())]
        cp_g(c).wait(); cp_u(c).wait(); cp_d(c).wait()
        for cond, cp in waits:
            pl.when(cond)(cp.wait)

        off = _off(c, FC1)
        xv = bf(x_v[0:R1 // 2, :])
        never = row8 + c < 0
        nt = FC1 // LANES
        res = []
        done = {}
        for m in range(2 * nt):
            w_v = wg_v if m < nt else wu_v
            w = w_v[:, pl.ds(pl.multiple_of(off + (m % nt) * LANES, LANES), LANES)]
            if m in done:
                w = jnp.concatenate([jnp.where(never, done[m], w[0:8, :]), w[8:, :]], axis=0)
            r = _dot(xv, bf(w))
            res.append(r)
            tok = pltpu.bitcast(r[0:8, :], U32)
            if m < UQ:
                done[m + P1_LAG] = prep_wq(m, uq[m], never, tok)
            elif m - 1 >= UQ and m - 1 < UQ + UO:
                toks = [pltpu.bitcast(r[rr:rr + 8, :], U32) for rr in range(0, R1, R1 // 4)]
                prep_wo(m - 1, uo[m - 1 - UQ], never, toks)
        g = jnp.concatenate(res[:nt], axis=1)
        u = jnp.concatenate(res[nt:], axis=1)
        h = (jnp.maximum(g, 0.0) * u).astype(BF16)
        b_v[0:R1, :] += _dot(h, bf(wd_v[rows(off, FC1), :]))
        return carry

    lax.fori_loop(1, n1, p1_body, 0)

    ngrp = MA // 16

    def p2_body(i, carry):
        ra = pl.multiple_of(i * MA, MA)
        rf = pl.multiple_of(R1 + i * MF, 16)
        k_v[:, 0:HALO, :] = k_v[:, MA:MA + HALO, :]
        v_v[:, 0:HALO, :] = v_v[:, MA:MA + HALO, :]
        gi = 0
        for c in range(n2):
            r, toks = ffn_chunk(bf(x_v[rows(rf, MF), :]), c * FC2, FC2)
            if c == 0:
                b_v[pl.ds(rf, MF), :] = r
                qkv(bf(x_v[rows(ra, MA), :]))
                continue
            b_v[pl.ds(rf, MF), :] += r
            for tg, ta, tb in TOKS:
                if gi < ngrp:
                    attn16(gi * 16, ra, toks[tg], toks[ta], toks[tb])
                    gi += 1
        a = _dot(bf(o_v[...]), bf(jnp.concatenate([wop_v[c] for c in range(NCH)], axis=1)))
        og = jnp.concatenate([og_v[...]] * NCH, axis=1)
        out_v[rows(ra, MA), :] = pltpu.bitcast((a + og * b_v[pl.ds(ra, MA), :]).astype(BF16), U32)
        cp_out(i).start()
        return carry

    lax.fori_loop(0, NIT, p2_body, 0)
    for i in range(NIT):
        cp_out(i).wait()


@jax.jit
def pallas_gated_mix__sliding_local_dilated__glu_gated_reglu__prompt_kernel(
    A_x: jax.Array,
    A_wqkv: jax.Array,
    A_wo: jax.Array,
    B_x: jax.Array,
    B_W_gate: jax.Array,
    B_W_up: jax.Array,
    B_W_down: jax.Array,
    gate_w: jax.Array,
):
    B, S, D = A_x.shape
    assert B == 1
    F = B_W_gate.shape[1]
    NCH = D // LANES
    MA = S // NIT
    n1 = F // FC1
    n_in = len(PEEL_COPIES) + 2 + 3 * (n1 - 1) + 2 * NAUX

    def kernel(*refs):
        def once(_, c):
            _kernel(*refs, S=S, D=D, F=F)
            return c

        lax.fori_loop(0, pl.program_id(0) + 1, once, 0)

    any_spec = pl.BlockSpec(memory_space=pl.ANY)
    return pl.pallas_call(
        kernel,
        grid=(1,),
        in_specs=[any_spec] * 7,
        out_specs=any_spec,
        out_shape=jax.ShapeDtypeStruct((B, S, D), A_x.dtype),
        scratch_shapes=[
            pltpu.VMEM((S // 2, D), U32),
            pltpu.VMEM(((D + LANES) // 2, 3 * D), U32),
            pltpu.VMEM((D // 2, D + LANES), U32),
            pltpu.VMEM((D // 2, F), U32),
            pltpu.VMEM((D // 2, F), U32),
            pltpu.VMEM((F // 2, D), U32),
            pltpu.VMEM((D,), BF16),
            pltpu.VMEM((NCH + 1, 3 * D // 2, LANES), U32),
            pltpu.VMEM((NCH + 1, D // 2, LANES), U32),
            pltpu.VMEM((UQ + UO, TMP_ROWS, LANES), U32),
            pltpu.VMEM((S, D), F32),
            pltpu.VMEM((NCH, MA, LANES), F32),
            pltpu.VMEM((NCH, HALO + MA + KV_PAD, LANES), F32),
            pltpu.VMEM((NCH, HALO + MA + KV_PAD, LANES), F32),
            pltpu.VMEM((MA // 2, D), U32),
            pltpu.VMEM((MA, LANES), F32),
            pltpu.VMEM((S // 2, D), U32),
            pltpu.SemaphoreType.DMA((n_in,)),
            pltpu.SemaphoreType.DMA((NIT,)),
        ],
        compiler_params=pltpu.CompilerParams(
            vmem_limit_bytes=100 * 1024 * 1024,
            disable_semaphore_checks=True,
            disable_bounds_checks=True,
        ),
    )(A_x, A_wqkv, A_wo, B_W_gate, B_W_up, B_W_down, gate_w)
```

```python
import jax
import jax.numpy as jnp
from jax import lax
import jax.experimental.pallas as pl
import jax.experimental.pallas.tpu as pltpu

H = 32
WIN = 8
DIL = 2
HALO = 16
LANES = 128
NEG = -1e9

R1 = 512
FC1 = 512
FC2 = 512
NIT = 8
PITCH = 17

TOKS = ((0, 1, 3), (0, 1, 3), (0, 2, 6))
DEADLINES = ((0, 2), (0, 4), (0, 2))
UQ = 5
UO = 2
NAUX = 4
P1_LAG = 2
TMP_ROWS = 552
KV_PAD = 0

PEEL_COPIES = (("x", 0, 256), ("g", 0, 256), ("x", 256, 512), ("u", 0, 256),
               ("g", 256, 512), ("u", 256, 512), ("d", 0, 512))
PEEL_STEPS = (
    ((0, 1), (("g", 0, 256, 0, 256),)),
    ((2,), (("g", 256, 512, 0, 256),)),
    ((3,), (("u", 0, 512, 0, 256), ("h", 0, 512, 0, 256))),
    ((4, 5), (("g", 0, 512, 256, 512), ("u", 0, 512, 256, 512), ("h", 0, 512, 256, 512))),
    ((6,), (("d", 0, 512, 0, 512),)),
)

F32 = jnp.float32
BF16 = jnp.bfloat16
U32 = jnp.uint32


def _dot(a, b):
    return jnp.dot(a, b, preferred_element_type=F32)


def _dot_nt(a, b):
    return lax.dot_general(a, b, (((1,), (1,)), ((), ())), preferred_element_type=F32)


def _kernel(x_hbm, wqkv_hbm, wo_hbm, wg_hbm, wu_hbm, wd_hbm, gw_hbm, out_hbm,
            x_v, wqkv_v, wo_v, wg_v, wu_v, wd_v, gw_v,
            wt_v, wop_v, tmp_v, b_v, q_v, k_v, v_v, o_v, og_v, out_v,
            sem_in, sem_out, *, S, D, F):
    NCH = D // LANES
    DH = D // H
    scale = DH ** -0.5
    n1 = F // FC1
    n2 = F // FC2
    MF = (S - R1) // NIT
    MA = S // NIT
    NU = 3 * NCH
    Q0 = 2 * UQ
    O0 = 2 * UO
    assert UQ * (n1 - 1) + UQ - 1 - Q0 >= NU - 1 and UO * (n1 - 1) + UO - 1 - O0 >= NCH - 1

    x_h = x_hbm.at[0].bitcast(U32)
    out_h = out_hbm.at[0].bitcast(U32)
    wqkv_h, wo_h, wg_h, wu_h, wd_h = (r.bitcast(U32) for r in (wqkv_hbm, wo_hbm, wg_hbm, wu_hbm, wd_hbm))

    def _off(c, n):
        return c * n if isinstance(c, int) else pl.multiple_of(c * n, n)

    def rows(start, n):
        if isinstance(start, int):
            return pl.ds(start // 2, n // 2)
        return pl.ds(pl.multiple_of(start // 2, 8), n // 2)

    def bf(v):
        return pltpu.bitcast(v, BF16)

    s_p = 0
    s_gw = len(PEEL_COPIES)
    s_xr = s_gw + 1
    s_w = s_xr + 1 - 3
    s_u = s_w + 3 * n1
    s_o = s_u + NAUX

    def cp_peel(n):
        kind, lo, hi = PEEL_COPIES[n]
        if kind == "x":
            sl = rows(lo, hi - lo)
            return pltpu.make_async_copy(x_h.at[sl, :], x_v.at[sl, :], sem_in.at[s_p + n])
        if kind == "d":
            sl = rows(lo, hi - lo)
            return pltpu.make_async_copy(wd_h.at[sl, :], wd_v.at[sl, :], sem_in.at[s_p + n])
        src, dst = (wg_h, wg_v) if kind == "g" else (wu_h, wu_v)
        sl = pl.ds(lo, hi - lo)
        return pltpu.make_async_copy(src.at[:, sl], dst.at[:, sl], sem_in.at[s_p + n])

    def cp_xr():
        sl = rows(R1, S - R1)
        return pltpu.make_async_copy(x_h.at[sl, :], x_v.at[sl, :], sem_in.at[s_xr])

    def cp_gw():
        return pltpu.make_async_copy(gw_hbm, gw_v, sem_in.at[s_gw])

    def cp_g(c):
        sl = pl.ds(_off(c, FC1), FC1)
        return pltpu.make_async_copy(wg_h.at[:, sl], wg_v.at[:, sl], sem_in.at[s_w + 3 * c])

    def cp_u(c):
        sl = pl.ds(_off(c, FC1), FC1)
        return pltpu.make_async_copy(wu_h.at[:, sl], wu_v.at[:, sl], sem_in.at[s_w + 3 * c + 1])

    def cp_d(c):
        sl = pl.ds(_off(c, FC1 // 2), FC1 // 2)
        return pltpu.make_async_copy(wd_h.at[sl, :], wd_v.at[sl, :], sem_in.at[s_w + 3 * c + 2])

    def cp_wq(t):
        sl = pl.ds(_off(t, D // NAUX // 2), D // NAUX // 2)
        return pltpu.make_async_copy(wqkv_h.at[sl, :], wqkv_v.at[sl, :], sem_in.at[s_u + t])

    def cp_wo(t):
        sl = pl.ds(_off(t, D // NAUX), D // NAUX)
        return pltpu.make_async_copy(wo_h.at[:, sl], wo_v.at[:, sl], sem_in.at[s_o + t])

    def cp_out(i):
        sl = pl.ds(_off(i, MA // 2), MA // 2)
        return pltpu.make_async_copy(out_v.at[sl, :], out_h.at[sl, :], sem_out.at[i])

    for n in range(len(PEEL_COPIES)):
        cp_peel(n).start()
    for c in range(1, n1):
        cp_g(c).start(); cp_u(c).start(); cp_d(c).start()
        if 0 <= c - 2 < NAUX:
            cp_wq(c - 2).start(); cp_wo(c - 2).start()
    cp_gw().start()
    cp_xr().start()

    lane8 = lax.broadcasted_iota(jnp.int32, (8, LANES), 1)
    odd = (lane8 & 1) == 1
    row8 = lax.broadcasted_iota(jnp.int32, (8, LANES), 0)

    def waits_for(never, toks, w):
        if not toks:
            return w
        top = [w[0:8, t * LANES:(t + 1) * LANES] for t in range(w.shape[1] // LANES)]
        top = [jnp.where(never, toks[t], v) if t in toks else v for t, v in enumerate(top)]
        return jnp.concatenate([jnp.concatenate(top, axis=1), w[8:, :]], axis=0)

    def tile(m, t):
        return m[0:8, t * LANES:(t + 1) * LANES]

    def permute_rows(slot, u32, dst, row0, col):
        for g in range(2 * H):
            tmp_v[slot, pl.ds((g // 2) * PITCH + (g % 2) * 8, 8), :] = u32[g * 8:(g + 1) * 8, :]
        for j in range(NCH):
            for e in range(2):
                base = row0 + (2 * j + e) * H
                if not isinstance(base, int):
                    base = pl.multiple_of(base, H)
                dst[col, pl.ds(base, H), :] = tmp_v[slot, pl.ds(8 * e + j, H, stride=PITCH), :]

    def after(never, tok, u32):
        return jnp.concatenate(
            [jnp.concatenate([jnp.where(never, tok, u32[r:r + 8, c:c + LANES])
                              for c in range(0, u32.shape[1], LANES)], axis=1)
             for r in range(0, u32.shape[0], 8)], axis=0)

    def prep_wq(slot, u, never, tok):
        kb, sec = u // 3, u % 3
        raw = wqkv_v[pl.ds(_off(kb, LANES // 2), LANES // 2), pl.ds(_off(sec, D), D)]
        u32 = pltpu.bitcast(bf(after(never, tok, raw)).T, U32)
        permute_rows(slot, u32, wt_v, _off(sec, D // 2), kb)
        tok = u32[56:64, :]
        for t in range(1, NCH):
            tok = tok | u32[t * 64 + 56:t * 64 + 64, :]
        return tok

    def prep_wo(slot, c, never, toks):
        n = D // 2 // len(toks)
        col = pl.ds(_off(c, LANES), LANES)
        u32 = jnp.concatenate([after(never, tok, wo_v[i * n:(i + 1) * n, col]) for i, tok in enumerate(toks)],
                              axis=0)
        permute_rows(slot, u32, wop_v, 0, c)

    def qkv(xa):
        for sec, dst, r0 in ((1, k_v, HALO), (0, q_v, 0), (2, v_v, HALO)):
            w = jnp.concatenate([wt_v[kb, sec * (D // 2):(sec + 1) * (D // 2), :] for kb in range(NCH)], axis=1)
            res = _dot_nt(xa, bf(w))
            for j in range(NCH):
                dst[j, r0:r0 + MA, :] = res[:, j * LANES:(j + 1) * LANES]

    def attn8(r, row0, never, tok, gate):
        sc = jnp.where(never, tok, scale)
        q = [q_v[j, r:r + 8, :] * sc for j in range(NCH)]
        logits = []
        for w in range(WIN):
            lo = HALO + r - DIL * w
            s = q[0] * k_v[0, lo:lo + 8, :]
            for j in range(1, NCH):
                s = s + q[j] * k_v[j, lo:lo + 8, :]
            s = s + pltpu.roll(s, 64, 1)
            s = s + jnp.where(odd, pltpu.roll(s, 1, 1), pltpu.roll(s, LANES - 1, 1))
            if r - DIL * w < 0:
                s = jnp.where(row8 + (row0 + r - DIL * w) >= 0, s, NEG)
            logits.append(s)
        m = logits[0]
        for w in range(1, WIN):
            m = jnp.maximum(m, logits[w])
        p = [jnp.exp(l - m) for l in logits]
        den = p[0]
        for w in range(1, WIN):
            den = den + p[w]
        inv = pl.reciprocal(den, approx=True)
        inv = inv * (2.0 - den * inv) * gate
        p = [pw * inv for pw in p]
        outs = []
        for j in range(NCH):
            acc = p[0] * v_v[j, HALO + r:HALO + r + 8, :]
            for w in range(1, WIN):
                lo = HALO + r - DIL * w
                acc = acc + p[w] * v_v[j, lo:lo + 8, :]
            outs.append(acc)
        return outs, pltpu.bitcast(inv, U32)

    def attn16(r, row0, never, tok_g, tok_a, tok_b):
        xg = bf(after(never, pltpu.bitcast(tok_g, U32), x_v[rows(row0 + r, 16), :])).astype(F32)
        z = jnp.sum(xg * gw_v[...].astype(F32).reshape(1, D), axis=-1, keepdims=True)
        th = 0.5 * jnp.tanh(jnp.broadcast_to(0.5 * z, (16, LANES)))
        gate = 0.5 + th
        og_v[r:r + 16, :] = 0.5 - th
        a, done_a = attn8(r, row0, never, tok_a, gate[0:8])
        b, done_b = attn8(r + 8, row0, never, tok_b, gate[8:16])
        for j in range(NCH):
            o_v[r // 2:r // 2 + 8, j * LANES:(j + 1) * LANES] = pltpu.bitcast(
                jnp.concatenate([a[j], b[j]], axis=0).astype(BF16), U32)
        return done_a, done_b

    k_v[:, MA:MA + HALO, :] = jnp.zeros((NCH, HALO, LANES), F32)
    v_v[:, MA:MA + HALO, :] = jnp.zeros((NCH, HALO, LANES), F32)
    wqkv_v[D // 2:, 0:D] = jnp.zeros((LANES // 2, D), U32)
    wo_v[:, D:] = jnp.zeros((D // 2, LANES), U32)

    parts = {}
    for waits, work in PEEL_STEPS:
        for n in waits:
            cp_peel(n).wait()
        for kind, r0, r1, c0, c1 in work:
            if kind in "gu":
                w_v = wg_v if kind == "g" else wu_v
                parts[kind, r0, c0] = (r1, c1, _dot(bf(x_v[rows(r0, r1 - r0), :]), bf(w_v[:, c0:c1])))
            elif kind == "h":
                def gather(kd):
                    cols = []
                    for cc in sorted({k[2] for k in parts if k[0] == kd and c0 <= k[2] < c1}):
                        rs = sorted(k[1] for k in parts if k[0] == kd and k[2] == cc)
                        cols.append(jnp.concatenate([parts[kd, r, cc][2] for r in rs], axis=0))
                    return jnp.concatenate(cols, axis=1)
                parts["h", 0, c0] = (r1, c1, (jnp.maximum(gather("g"), 0.0) * gather("u")).astype(BF16))
            else:
                h = jnp.concatenate([parts[k][2] for k in sorted(parts) if k[0] == "h" and c0 <= k[2] < c1], axis=1)
                r = _dot(h, bf(wd_v[rows(c0, c1 - c0), :]))
                if c0 == 0:
                    b_v[0:R1, :] = r
                else:
                    b_v[0:R1, :] += r

    def p1_body(c, carry):
        uq = [UQ * c + t - Q0 for t in range(UQ)]
        uo = [UO * c + t - O0 for t in range(UO)]
        uq = [jnp.where(jnp.logical_and(u >= 0, u < NU), u, NU) for u in uq]
        uo = [jnp.where(jnp.logical_and(u >= 0, u < NCH), u, NCH) for u in uo]
        aux = jnp.logical_and(c >= 2, c < 2 + NAUX)
        ta = jnp.clip(c - 2, 0, NAUX - 1)
        last = c == n1 - 1
        waits = [(aux, cp_wq(ta)), (aux, cp_wo(ta)), (last, cp_gw()), (last, cp_xr())]
        cp_g(c).wait(); cp_u(c).wait(); cp_d(c).wait()
        for cond, cp in waits:
            pl.when(cond)(cp.wait)

        off = _off(c, FC1)
        xv = bf(x_v[0:R1 // 2, :])
        never = row8 + c < 0
        nt = FC1 // LANES
        res = []
        done = {}
        for m in range(2 * nt):
            w_v = wg_v if m < nt else wu_v
            w = w_v[:, pl.ds(pl.multiple_of(off + (m % nt) * LANES, LANES), LANES)]
            r = _dot(xv, bf(waits_for(never, {0: done[m]} if m in done else None, w)))
            res.append(r)
            tok = pltpu.bitcast(r[0:8, :], U32)
            if m < UQ:
                done[m + P1_LAG] = prep_wq(m, uq[m], never, tok)
            elif m - 1 >= UQ and m - 1 < UQ + UO:
                toks = [pltpu.bitcast(r[rr:rr + 8, :], U32) for rr in range(0, R1, R1 // 4)]
                prep_wo(m - 1, uo[m - 1 - UQ], never, toks)
        g = jnp.concatenate(res[:nt], axis=1)
        u = jnp.concatenate(res[nt:], axis=1)
        h = (jnp.maximum(g, 0.0) * u).astype(BF16)
        b_v[0:R1, :] += _dot(h, bf(wd_v[rows(off, FC1), :]))
        return carry

    lax.fori_loop(1, n1, p1_body, 0)

    def p2_body(i, carry):
        ra = pl.multiple_of(i * MA, MA)
        rf = pl.multiple_of(R1 + i * MF, 16)
        k_v[:, 0:HALO, :] = k_v[:, MA:MA + HALO, :]
        v_v[:, 0:HALO, :] = v_v[:, MA:MA + HALO, :]
        never = row8 + i < 0
        groups = iter(range(0, MA, 16))

        def attn_group(m, k):
            r = next(groups, None)
            if r is None:
                return None
            return dict(zip(DEADLINES[k], attn16(r, ra, never, *(tile(m, t) for t in TOKS[k]))))

        dl = None
        for c in range(n2):
            off = c * FC2
            xv = bf(x_v[rows(rf, MF), :])
            g = _dot(xv, bf(waits_for(never, dl, wg_v[:, off:off + FC2])))
            dl = attn_group(g, 0) if c > 0 else None
            u = _dot(xv, bf(waits_for(never, dl, wu_v[:, off:off + FC2])))
            dl = attn_group(u, 1) if c > 0 else None
            h = (jnp.maximum(g, 0.0) * u).astype(BF16)
            r = _dot(h, bf(waits_for(never, dl, wd_v[rows(off, FC2), :])))
            if c == 0:
                b_v[pl.ds(rf, MF), :] = r
                qkv(bf(x_v[rows(ra, MA), :]))
            else:
                b_v[pl.ds(rf, MF), :] += r
                dl = attn_group(r, 2)
        a = _dot(bf(o_v[...]), bf(jnp.concatenate([wop_v[c] for c in range(NCH)], axis=1)))
        og = jnp.concatenate([og_v[...]] * NCH, axis=1)
        out_v[rows(ra, MA), :] = pltpu.bitcast((a + og * b_v[pl.ds(ra, MA), :]).astype(BF16), U32)
        cp_out(i).start()
        return carry

    lax.fori_loop(0, NIT, p2_body, 0)
    for i in range(NIT):
        cp_out(i).wait()


@jax.jit
def pallas_gated_mix__sliding_local_dilated__glu_gated_reglu__prompt_kernel(
    A_x: jax.Array,
    A_wqkv: jax.Array,
    A_wo: jax.Array,
    B_x: jax.Array,
    B_W_gate: jax.Array,
    B_W_up: jax.Array,
    B_W_down: jax.Array,
    gate_w: jax.Array,
):
    B, S, D = A_x.shape
    assert B == 1
    F = B_W_gate.shape[1]
    NCH = D // LANES
    MA = S // NIT
    n1 = F // FC1
    n_in = len(PEEL_COPIES) + 2 + 3 * (n1 - 1) + 2 * NAUX

    def kernel(*refs):
        def once(_, c):
            _kernel(*refs, S=S, D=D, F=F)
            return c

        lax.fori_loop(0, pl.program_id(0) + 1, once, 0)

    any_spec = pl.BlockSpec(memory_space=pl.ANY)
    return pl.pallas_call(
        kernel,
        grid=(1,),
        in_specs=[any_spec] * 7,
        out_specs=any_spec,
        out_shape=jax.ShapeDtypeStruct((B, S, D), A_x.dtype),
        scratch_shapes=[
            pltpu.VMEM((S // 2, D), U32),
            pltpu.VMEM(((D + LANES) // 2, 3 * D), U32),
            pltpu.VMEM((D // 2, D + LANES), U32),
            pltpu.VMEM((D // 2, F), U32),
            pltpu.VMEM((D // 2, F), U32),
            pltpu.VMEM((F // 2, D), U32),
            pltpu.VMEM((D,), BF16),
            pltpu.VMEM((NCH + 1, 3 * D // 2, LANES), U32),
            pltpu.VMEM((NCH + 1, D // 2, LANES), U32),
            pltpu.VMEM((UQ + UO, TMP_ROWS, LANES), U32),
            pltpu.VMEM((S, D), F32),
            pltpu.VMEM((NCH, MA, LANES), F32),
            pltpu.VMEM((NCH, HALO + MA + KV_PAD, LANES), F32),
            pltpu.VMEM((NCH, HALO + MA + KV_PAD, LANES), F32),
            pltpu.VMEM((MA // 2, D), U32),
            pltpu.VMEM((MA, LANES), F32),
            pltpu.VMEM((S // 2, D), U32),
            pltpu.SemaphoreType.DMA((n_in,)),
            pltpu.SemaphoreType.DMA((NIT,)),
        ],
        compiler_params=pltpu.CompilerParams(
            vmem_limit_bytes=100 * 1024 * 1024,
            disable_semaphore_checks=True,
            disable_bounds_checks=True,
        ),
    )(A_x, A_wqkv, A_wo, B_W_gate, B_W_up, B_W_down, gate_w)
```

```python
import jax
import jax.numpy as jnp
from jax import lax
import jax.experimental.pallas as pl
import jax.experimental.pallas.tpu as pltpu

H = 32
WIN = 8
DIL = 2
HALO = 16
LANES = 128
NEG = -1e9
LOG2E = 1.4426950408889634

R1 = 512
FC1 = 512
FC2 = 512
NIT = 8
PITCH = 17

TOKS = ((0, 1, 3), (0, 1, 3), (0, 2, 6))
DEADLINES = ((0, 2), (0, 4), (0, 2))
UQ = 5
UO = 2
NAUX = 4
P1_LAG = 2
EXP2 = False
QKV_ORDER = (1, 0, 2)
QKV_AFTER = 0
P1_GET_STEP = 8
OUT_SPLIT = (0, 1024)
WO_TILES = ((0, 1), (3, 4))
TMP_ROWS = 552
KV_PAD = 0

PEEL_COPIES = (("x", 0, 128), ("g", 0, 128), ("x", 128, 256), ("g", 128, 256), ("x", 256, 512),
               ("u", 0, 256), ("g", 256, 512), ("u", 256, 512), ("d", 0, 512))
PEEL_STEPS = (
    ((0, 1), (("g", 0, 128, 0, 128),)),
    ((2,), (("g", 128, 256, 0, 128),)),
    ((3,), (("g", 0, 256, 128, 256),)),
    ((4,), (("g", 256, 512, 0, 128), ("g", 256, 512, 128, 256))),
    ((5,), (("u", 0, 512, 0, 256), ("h", 0, 512, 0, 256))),
    ((6, 7), (("g", 0, 512, 256, 512), ("u", 0, 512, 256, 512), ("h", 0, 512, 256, 512))),
    ((8,), (("d", 0, 512, 0, 512),)),
)

F32 = jnp.float32
BF16 = jnp.bfloat16
U32 = jnp.uint32


def _dot(a, b):
    return jnp.dot(a, b, preferred_element_type=F32)


def _dot_nt(a, b):
    return lax.dot_general(a, b, (((1,), (1,)), ((), ())), preferred_element_type=F32)


def _kernel(x_hbm, wqkv_hbm, wo_hbm, wg_hbm, wu_hbm, wd_hbm, gw_hbm, out_hbm,
            x_v, wqkv_v, wo_v, wg_v, wu_v, wd_v, gw_v,
            wt_v, wop_v, tmp_v, b_v, q_v, k_v, v_v, o_v, og_v, out_v,
            sem_in, sem_out, *, S, D, F):
    NCH = D // LANES
    DH = D // H
    scale = DH ** -0.5
    n1 = F // FC1
    n2 = F // FC2
    MF = (S - R1) // NIT
    MA = S // NIT
    NU = 3 * NCH
    Q0 = 2 * UQ
    O0 = 2 * UO
    assert UQ * (n1 - 1) + UQ - 1 - Q0 >= NU - 1 and UO * (n1 - 1) + UO - 1 - O0 >= NCH - 1

    x_h = x_hbm.at[0].bitcast(U32)
    out_h = out_hbm.at[0].bitcast(U32)
    wqkv_h, wo_h, wg_h, wu_h, wd_h = (r.bitcast(U32) for r in (wqkv_hbm, wo_hbm, wg_hbm, wu_hbm, wd_hbm))

    def _off(c, n):
        return c * n if isinstance(c, int) else pl.multiple_of(c * n, n)

    def rows(start, n):
        if isinstance(start, int):
            return pl.ds(start // 2, n // 2)
        return pl.ds(pl.multiple_of(start // 2, 8), n // 2)

    def bf(v):
        return pltpu.bitcast(v, BF16)

    s_p = 0
    s_gw = len(PEEL_COPIES)
    s_xr = s_gw + 1
    s_w = s_xr + 1 - 3
    s_u = s_w + 3 * n1
    s_o = s_u + NAUX

    def cp_peel(n):
        kind, lo, hi = PEEL_COPIES[n]
        if kind == "x":
            sl = rows(lo, hi - lo)
            return pltpu.make_async_copy(x_h.at[sl, :], x_v.at[sl, :], sem_in.at[s_p + n])
        if kind == "d":
            sl = rows(lo, hi - lo)
            return pltpu.make_async_copy(wd_h.at[sl, :], wd_v.at[sl, :], sem_in.at[s_p + n])
        src, dst = (wg_h, wg_v) if kind == "g" else (wu_h, wu_v)
        sl = pl.ds(lo, hi - lo)
        return pltpu.make_async_copy(src.at[:, sl], dst.at[:, sl], sem_in.at[s_p + n])

    def cp_xr():
        sl = rows(R1, S - R1)
        return pltpu.make_async_copy(x_h.at[sl, :], x_v.at[sl, :], sem_in.at[s_xr])

    def cp_gw():
        return pltpu.make_async_copy(gw_hbm, gw_v, sem_in.at[s_gw])

    def cp_g(c):
        sl = pl.ds(_off(c, FC1), FC1)
        return pltpu.make_async_copy(wg_h.at[:, sl], wg_v.at[:, sl], sem_in.at[s_w + 3 * c])

    def cp_u(c):
        sl = pl.ds(_off(c, FC1), FC1)
        return pltpu.make_async_copy(wu_h.at[:, sl], wu_v.at[:, sl], sem_in.at[s_w + 3 * c + 1])

    def cp_d(c):
        sl = pl.ds(_off(c, FC1 // 2), FC1 // 2)
        return pltpu.make_async_copy(wd_h.at[sl, :], wd_v.at[sl, :], sem_in.at[s_w + 3 * c + 2])

    def cp_wq(t):
        sl = pl.ds(_off(t, D // NAUX // 2), D // NAUX // 2)
        return pltpu.make_async_copy(wqkv_h.at[sl, :], wqkv_v.at[sl, :], sem_in.at[s_u + t])

    def cp_wo(t):
        sl = pl.ds(_off(t, D // NAUX), D // NAUX)
        return pltpu.make_async_copy(wo_h.at[:, sl], wo_v.at[:, sl], sem_in.at[s_o + t])

    def cp_out(i, t):
        sl = pl.ds(_off(i, MA // 2), MA // 2)
        c0, c1 = OUT_SPLIT[t], OUT_SPLIT[t + 1]
        return pltpu.make_async_copy(out_v.at[sl, c0:c1], out_h.at[sl, c0:c1],
                                     sem_out.at[i * (len(OUT_SPLIT) - 1) + t])

    for n in range(len(PEEL_COPIES)):
        cp_peel(n).start()

    def issue(c, carry):
        cp_g(c).start(); cp_u(c).start(); cp_d(c).start()

        @pl.when(jnp.logical_and(c >= 2, c < 2 + NAUX))
        def _():
            cp_wq(c - 2).start(); cp_wo(c - 2).start()
        return carry

    lax.fori_loop(1, n1, issue, 0)
    cp_gw().start()
    cp_xr().start()

    lane8 = lax.broadcasted_iota(jnp.int32, (8, LANES), 1)
    odd = (lane8 & 1) == 1
    row8 = lax.broadcasted_iota(jnp.int32, (8, LANES), 0)

    def waits_for(never, toks, w):
        if not toks:
            return w
        top = [w[0:8, t * LANES:(t + 1) * LANES] for t in range(w.shape[1] // LANES)]
        top = [jnp.where(never, toks[t], v) if t in toks else v for t, v in enumerate(top)]
        return jnp.concatenate([jnp.concatenate(top, axis=1), w[8:, :]], axis=0)

    def tile(m, t):
        return m[0:8, t * LANES:(t + 1) * LANES]

    def permute_put(slot, u32):
        for g in range(2 * H):
            tmp_v[slot, pl.ds((g // 2) * PITCH + (g % 2) * 8, 8), :] = u32[g * 8:(g + 1) * 8, :]

    def permute_get(slot, dst, row0, col, never, toks):
        for n in range(2 * NCH * H // 8):
            je, a = divmod(n, H // 8)
            base = row0 + n * 8
            if not isinstance(base, int):
                base = pl.multiple_of(base, 8)
            val = tmp_v[slot, pl.ds(8 * (je % 2) + je // 2 + a * 8 * PITCH, 8, stride=PITCH), :]
            if toks:
                val = jnp.where(never, toks[n * len(toks) // (2 * NCH * H // 8)], val)
            dst[col, pl.ds(base, 8), :] = val

    def after(never, tok, u32):
        return jnp.concatenate(
            [jnp.concatenate([jnp.where(never, tok, u32[r:r + 8, c:c + LANES])
                              for c in range(0, u32.shape[1], LANES)], axis=1)
             for r in range(0, u32.shape[0], 8)], axis=0)

    def prep_wq_put(slot, u, never, tok):
        kb, sec = u // 3, u % 3
        raw = wqkv_v[pl.ds(_off(kb, LANES // 2), LANES // 2), pl.ds(_off(sec, D), D)]
        u32 = pltpu.bitcast(bf(after(never, tok, raw)).T, U32)
        permute_put(slot, u32)
        tok = u32[56:64, :]
        for t in range(1, NCH):
            tok = tok | u32[t * 64 + 56:t * 64 + 64, :]
        return tok

    def prep_wq_get(slot, u, never, toks):
        permute_get(slot, wt_v, _off(u % 3, D // 2), u // 3, never, toks)

    def prep_wo_put(slot, c, never, toks):
        n = D // 2 // len(toks)
        col = pl.ds(_off(c, LANES), LANES)
        permute_put(slot, jnp.concatenate(
            [after(never, tok, wo_v[i * n:(i + 1) * n, col]) for i, tok in enumerate(toks)], axis=0))

    def qkv(xa):
        for sec in QKV_ORDER:
            dst, r0 = ((q_v, 0), (k_v, HALO), (v_v, HALO))[sec]
            w = jnp.concatenate([wt_v[kb, sec * (D // 2):(sec + 1) * (D // 2), :] for kb in range(NCH)], axis=1)
            res = _dot_nt(xa, bf(w))
            for j in range(NCH):
                dst[j, r0:r0 + MA, :] = res[:, j * LANES:(j + 1) * LANES]

    def attn8(r, row0, never, tok, gate):
        sc = jnp.where(never, tok, scale * (LOG2E if EXP2 else 1.0))
        q = [q_v[j, r:r + 8, :] * sc for j in range(NCH)]
        logits = []
        for w in range(WIN):
            lo = HALO + r - DIL * w
            s = q[0] * k_v[0, lo:lo + 8, :]
            for j in range(1, NCH):
                s = s + q[j] * k_v[j, lo:lo + 8, :]
            s = s + pltpu.roll(s, 64, 1)
            s = s + jnp.where(odd, pltpu.roll(s, 1, 1), pltpu.roll(s, LANES - 1, 1))
            if r - DIL * w < 0:
                s = jnp.where(row8 + (row0 + r - DIL * w) >= 0, s, NEG * (LOG2E if EXP2 else 1.0))
            logits.append(s)
        m = logits[0]
        for w in range(1, WIN):
            m = jnp.maximum(m, logits[w])
        p = [(jnp.exp2 if EXP2 else jnp.exp)(l - m) for l in logits]
        den = p[0]
        for w in range(1, WIN):
            den = den + p[w]
        inv = pl.reciprocal(den, approx=True)
        inv = inv * (2.0 - den * inv) * gate
        p = [pw * inv for pw in p]
        outs = []
        for j in range(NCH):
            acc = p[0] * v_v[j, HALO + r:HALO + r + 8, :]
            for w in range(1, WIN):
                lo = HALO + r - DIL * w
                acc = acc + p[w] * v_v[j, lo:lo + 8, :]
            outs.append(acc)
        return outs, pltpu.bitcast(inv, U32)

    def attn16(r, row0, never, tok_g, tok_a, tok_b):
        xg = bf(after(never, pltpu.bitcast(tok_g, U32), x_v[rows(row0 + r, 16), :])).astype(F32)
        z = jnp.sum(xg * gw_v[...].astype(F32).reshape(1, D), axis=-1, keepdims=True)
        th = 0.5 * jnp.tanh(jnp.broadcast_to(0.5 * z, (16, LANES)))
        gate = 0.5 + th
        og_v[r:r + 16, :] = 0.5 - th
        a, done_a = attn8(r, row0, never, tok_a, gate[0:8])
        b, done_b = attn8(r + 8, row0, never, tok_b, gate[8:16])
        for j in range(NCH):
            o_v[r // 2:r // 2 + 8, j * LANES:(j + 1) * LANES] = pltpu.bitcast(
                jnp.concatenate([a[j], b[j]], axis=0).astype(BF16), U32)
        return done_a, done_b

    def clear(j, carry):
        k_v[j, MA:MA + HALO, :] = jnp.zeros((HALO, LANES), F32)
        v_v[j, MA:MA + HALO, :] = jnp.zeros((HALO, LANES), F32)
        wqkv_v[pl.ds(pl.multiple_of(D // 2 + j * 8, 8), 8), 0:D] = jnp.zeros((8, D), U32)
        wo_v[pl.ds(_off(j, LANES // 2), LANES // 2), D:] = jnp.zeros((LANES // 2, LANES), U32)
        return carry

    lax.fori_loop(0, NCH, clear, 0)

    parts = {}
    for waits, work in PEEL_STEPS:
        for n in waits:
            cp_peel(n).wait()
        for kind, r0, r1, c0, c1 in work:
            if kind in "gu":
                w_v = wg_v if kind == "g" else wu_v
                parts[kind, r0, c0] = (r1, c1, _dot(bf(x_v[rows(r0, r1 - r0), :]), bf(w_v[:, c0:c1])))
            elif kind == "h":
                def gather(kd):
                    cols = []
                    for cc in sorted({k[2] for k in parts if k[0] == kd and c0 <= k[2] < c1}):
                        rs = sorted(k[1] for k in parts if k[0] == kd and k[2] == cc)
                        cols.append(jnp.concatenate([parts[kd, r, cc][2] for r in rs], axis=0))
                    return jnp.concatenate(cols, axis=1)
                parts["h", 0, c0] = (r1, c1, (jnp.maximum(gather("g"), 0.0) * gather("u")).astype(BF16))
            else:
                h = jnp.concatenate([parts[k][2] for k in sorted(parts) if k[0] == "h" and c0 <= k[2] < c1], axis=1)
                r = _dot(h, bf(wd_v[rows(c0, c1 - c0), :]))
                if c0 == 0:
                    b_v[0:R1, :] = r
                else:
                    b_v[0:R1, :] += r

    def p1_body(c, carry):
        aux = jnp.logical_and(c >= 2, c < 2 + NAUX)
        ta = jnp.clip(c - 2, 0, NAUX - 1)
        cp_g(c).wait(); cp_u(c).wait(); cp_d(c).wait()
        pl.when(aux)(cp_wq(ta).wait)
        pl.when(aux)(cp_wo(ta).wait)
        uq = [UQ * c + t - Q0 for t in range(UQ)]
        uo = [UO * c + t - O0 for t in range(UO)]
        uq = [jnp.where(jnp.logical_and(u >= 0, u < NU), u, NU) for u in uq]
        uo = [jnp.where(jnp.logical_and(u >= 0, u < NCH), u, NCH) for u in uo]
        off = _off(c, FC1)
        xv = bf(x_v[0:R1 // 2, :])
        never = row8 + c < 0
        nt = FC1 // LANES
        res = []
        done = {}
        for m in range(2 * nt):
            w_v = wg_v if m < nt else wu_v
            w = w_v[:, pl.ds(pl.multiple_of(off + (m % nt) * LANES, LANES), LANES)]
            r = _dot(xv, bf(waits_for(never, {0: done[m]} if m in done else None, w)))
            res.append(r)
            if m < UQ:
                done[m + P1_LAG] = prep_wq_put(m, uq[m], never, pltpu.bitcast(r[0:8, :], U32))
            if 0 <= m - P1_LAG < UQ:
                toks = [pltpu.bitcast(r[rr:rr + 8, :], U32) for rr in range(0, R1, P1_GET_STEP)] if P1_GET_STEP else None
                prep_wq_get(m - P1_LAG, uq[m - P1_LAG], never, toks)
        g = jnp.concatenate(res[:nt], axis=1)
        u = jnp.concatenate(res[nt:], axis=1)
        h = (jnp.maximum(g, 0.0) * u).astype(BF16)
        r = _dot(h, bf(wd_v[rows(off, FC1), :]))
        b_v[0:R1, :] += r
        for t in range(UO):
            toks = [pltpu.bitcast(r[rr:rr + 8, tt * LANES:(tt + 1) * LANES], U32)
                    for tt in WO_TILES[t] for rr in range(0, R1, R1 // 4)]
            prep_wo_put(UQ + t, uo[t], never, toks)
            tt = WO_TILES[t][-1] + 1
            toks = ([pltpu.bitcast(r[rr:rr + 8, tt * LANES:(tt + 1) * LANES], U32)
                     for rr in range(0, R1, P1_GET_STEP)] if P1_GET_STEP else None)
            permute_get(UQ + t, wop_v, 0, uo[t], never, toks)
        return carry

    lax.fori_loop(1, n1, p1_body, 0)
    cp_gw().wait()
    cp_xr().wait()

    def p2_body(i, carry):
        ra = pl.multiple_of(i * MA, MA)
        rf = pl.multiple_of(R1 + i * MF, 16)
        k_v[:, 0:HALO, :] = k_v[:, MA:MA + HALO, :]
        v_v[:, 0:HALO, :] = v_v[:, MA:MA + HALO, :]
        never = row8 + i < 0
        groups = iter(range(0, MA, 16))

        def attn_group(m, k):
            r = next(groups, None)
            if r is None:
                return None
            return dict(zip(DEADLINES[k], attn16(r, ra, never, *(tile(m, t) for t in TOKS[k]))))

        dl = None
        if QKV_AFTER < 0:
            qkv(bf(x_v[rows(ra, MA), :]))
        for c in range(n2):
            off = c * FC2
            xv = bf(x_v[rows(rf, MF), :])
            g = _dot(xv, bf(waits_for(never, dl, wg_v[:, off:off + FC2])))
            dl = attn_group(g, 0) if c > QKV_AFTER else None
            u = _dot(xv, bf(waits_for(never, dl, wu_v[:, off:off + FC2])))
            dl = attn_group(u, 1) if c > QKV_AFTER else None
            h = (jnp.maximum(g, 0.0) * u).astype(BF16)
            r = _dot(h, bf(waits_for(never, dl, wd_v[rows(off, FC2), :])))
            if c == 0:
                b_v[pl.ds(rf, MF), :] = r
            else:
                b_v[pl.ds(rf, MF), :] += r
            if c == QKV_AFTER:
                qkv(bf(x_v[rows(ra, MA), :]))
            dl = attn_group(r, 2) if c > QKV_AFTER else None
        for t in range(len(OUT_SPLIT) - 1):
            c0, c1 = OUT_SPLIT[t], OUT_SPLIT[t + 1]
            tiles = range(c0 // LANES, c1 // LANES)
            a = _dot(bf(o_v[...]), bf(jnp.concatenate([wop_v[c] for c in tiles], axis=1)))
            og = jnp.concatenate([og_v[...]] * len(tiles), axis=1)
            out_v[rows(ra, MA), c0:c1] = pltpu.bitcast(
                (a + og * b_v[pl.ds(ra, MA), c0:c1]).astype(BF16), U32)
            cp_out(i, t).start()
        return carry

    lax.fori_loop(0, NIT, p2_body, 0)
    for i in range(NIT):
        for t in range(len(OUT_SPLIT) - 1):
            cp_out(i, t).wait()


@jax.jit
def pallas_gated_mix__sliding_local_dilated__glu_gated_reglu__prompt_kernel(
    A_x: jax.Array,
    A_wqkv: jax.Array,
    A_wo: jax.Array,
    B_x: jax.Array,
    B_W_gate: jax.Array,
    B_W_up: jax.Array,
    B_W_down: jax.Array,
    gate_w: jax.Array,
):
    B, S, D = A_x.shape
    assert B == 1
    F = B_W_gate.shape[1]
    NCH = D // LANES
    MA = S // NIT
    n1 = F // FC1
    n_in = len(PEEL_COPIES) + 2 + 3 * (n1 - 1) + 2 * NAUX

    def kernel(*refs):
        def once(_, c):
            _kernel(*refs, S=S, D=D, F=F)
            return c

        lax.fori_loop(0, pl.program_id(0) + 1, once, 0)

    any_spec = pl.BlockSpec(memory_space=pl.ANY)
    return pl.pallas_call(
        kernel,
        grid=(1,),
        in_specs=[any_spec] * 7,
        out_specs=any_spec,
        out_shape=jax.ShapeDtypeStruct((B, S, D), A_x.dtype),
        scratch_shapes=[
            pltpu.VMEM((S // 2, D), U32),
            pltpu.VMEM(((D + LANES) // 2, 3 * D), U32),
            pltpu.VMEM((D // 2, D + LANES), U32),
            pltpu.VMEM((D // 2, F), U32),
            pltpu.VMEM((D // 2, F), U32),
            pltpu.VMEM((F // 2, D), U32),
            pltpu.VMEM((D,), BF16),
            pltpu.VMEM((NCH + 1, 3 * D // 2, LANES), U32),
            pltpu.VMEM((NCH + 1, D // 2, LANES), U32),
            pltpu.VMEM((UQ + UO, TMP_ROWS, LANES), U32),
            pltpu.VMEM((S, D), F32),
            pltpu.VMEM((NCH, MA, LANES), F32),
            pltpu.VMEM((NCH, HALO + MA + KV_PAD, LANES), F32),
            pltpu.VMEM((NCH, HALO + MA + KV_PAD, LANES), F32),
            pltpu.VMEM((MA // 2, D), U32),
            pltpu.VMEM((MA, LANES), F32),
            pltpu.VMEM((S // 2, D), U32),
            pltpu.SemaphoreType.DMA((n_in,)),
            pltpu.SemaphoreType.DMA((NIT * (len(OUT_SPLIT) - 1),)),
        ],
        compiler_params=pltpu.CompilerParams(
            vmem_limit_bytes=100 * 1024 * 1024,
            disable_semaphore_checks=True,
            disable_bounds_checks=True,
        ),
    )(A_x, A_wqkv, A_wo, B_W_gate, B_W_up, B_W_down, gate_w)
```

```python
import jax
import jax.numpy as jnp
from jax import lax
import jax.experimental.pallas as pl
import jax.experimental.pallas.tpu as pltpu

H = 32
WIN = 8
DIL = 2
HALO = 16
LANES = 128
NEG = -1e9
LOG2E = 1.4426950408889634

R1 = 512
FC1 = 512
FC2 = 512
NIT = 8
PITCH = 17

TOKS = ((0, 1, 3), (0, 1, 3), (0, 2, 6))
DEADLINES = ((0, 2), (0, 4), (0, 2))
UQ = 5
UO = 2
NAUX = 4
P1_LAG = 2
NATIVE = False
EXP2 = True
QKV_ORDER = (1, 0, 2)
QKV_AFTER = -1
P1_GET_STEP = 8
OUT_SPLIT = (0, 1024)
WO_TILES = ((0, 1), (3, 4))
TMP_ROWS = 552
KV_PAD = 0

PEEL_COPIES = (("x", 0, 128), ("g", 0, 128), ("x", 128, 256), ("g", 128, 256), ("x", 256, 512),
               ("u", 0, 256), ("g", 256, 512), ("u", 256, 512), ("d", 0, 512))
PEEL_STEPS = (
    ((0, 1), (("g", 0, 128, 0, 128),)),
    ((2,), (("g", 128, 256, 0, 128),)),
    ((3,), (("g", 0, 256, 128, 256),)),
    ((4,), (("g", 256, 512, 0, 128), ("g", 256, 512, 128, 256))),
    ((5,), (("u", 0, 512, 0, 256), ("h", 0, 512, 0, 256))),
    ((6, 7), (("g", 0, 512, 256, 512), ("u", 0, 512, 256, 512), ("h", 0, 512, 256, 512))),
    ((8,), (("d", 0, 512, 0, 512),)),
)

F32 = jnp.float32
BF16 = jnp.bfloat16
U32 = jnp.uint32


def _dot(a, b):
    return jnp.dot(a, b, preferred_element_type=F32)


def _dot_nt(a, b):
    return lax.dot_general(a, b, (((1,), (1,)), ((), ())), preferred_element_type=F32)


def _kernel(x_hbm, wqkv_hbm, wo_hbm, wg_hbm, wu_hbm, wd_hbm, gw_hbm, out_hbm,
            x_v, wqkv_v, wo_v, wg_v, wu_v, wd_v, gw_v,
            wt_v, wop_v, tmp_v, b_v, q_v, k_v, v_v, o_v, og_v, out_v,
            sem_in, sem_out, *, S, D, F):
    NCH = D // LANES
    DH = D // H
    scale = DH ** -0.5
    n1 = F // FC1
    n2 = F // FC2
    MF = (S - R1) // NIT
    MA = S // NIT
    NU = 3 * NCH
    Q0 = 2 * UQ
    O0 = 2 * UO
    assert UQ * (n1 - 1) + UQ - 1 - Q0 >= NU - 1 and UO * (n1 - 1) + UO - 1 - O0 >= NCH - 1

    PK = 2 if NATIVE else 1
    hb = (lambda r: r.bitcast(U32)) if NATIVE else (lambda r: r)
    x_h = hb(x_hbm.at[0])
    out_h = hb(out_hbm.at[0])
    wqkv_h, wo_h, wg_h, wu_h, wd_h = (hb(r) for r in (wqkv_hbm, wo_hbm, wg_hbm, wu_hbm, wd_hbm))

    def _off(c, n):
        return c * n if isinstance(c, int) else pl.multiple_of(c * n, n)

    def rows(start, n, i=0, step=0):
        if isinstance(i, int):
            return pl.ds((start + i * step) // PK, n // PK)
        return pl.ds(pl.multiple_of(start // PK + i * (step // PK), 16 // PK), n // PK)

    def pk(v):
        return v if NATIVE else pltpu.bitcast(v, U32)

    def bf(v):
        return pltpu.bitcast(v, BF16)

    s_p = 0
    s_gw = len(PEEL_COPIES)
    s_xr = s_gw + 1
    s_w = s_xr + 1 - 3
    s_u = s_w + 3 * n1
    s_o = s_u + NAUX

    def cp_peel(n):
        kind, lo, hi = PEEL_COPIES[n]
        if kind == "x":
            sl = rows(lo, hi - lo)
            return pltpu.make_async_copy(x_h.at[sl, :], x_v.at[sl, :], sem_in.at[s_p + n])
        if kind == "d":
            sl = rows(lo, hi - lo)
            return pltpu.make_async_copy(wd_h.at[sl, :], wd_v.at[sl, :], sem_in.at[s_p + n])
        src, dst = (wg_h, wg_v) if kind == "g" else (wu_h, wu_v)
        sl = pl.ds(lo, hi - lo)
        return pltpu.make_async_copy(src.at[:, sl], dst.at[:, sl], sem_in.at[s_p + n])

    def cp_xr():
        sl = rows(R1, S - R1)
        return pltpu.make_async_copy(x_h.at[sl, :], x_v.at[sl, :], sem_in.at[s_xr])

    def cp_gw():
        return pltpu.make_async_copy(gw_hbm, gw_v, sem_in.at[s_gw])

    def cp_g(c):
        sl = pl.ds(_off(c, FC1), FC1)
        return pltpu.make_async_copy(wg_h.at[:, sl], wg_v.at[:, sl], sem_in.at[s_w + 3 * c])

    def cp_u(c):
        sl = pl.ds(_off(c, FC1), FC1)
        return pltpu.make_async_copy(wu_h.at[:, sl], wu_v.at[:, sl], sem_in.at[s_w + 3 * c + 1])

    def cp_d(c):
        sl = rows(0, FC1, c, FC1)
        return pltpu.make_async_copy(wd_h.at[sl, :], wd_v.at[sl, :], sem_in.at[s_w + 3 * c + 2])

    def cp_wq(t):
        sl = rows(0, D // NAUX, t, D // NAUX)
        return pltpu.make_async_copy(wqkv_h.at[sl, :], wqkv_v.at[sl, :], sem_in.at[s_u + t])

    def cp_wo(t):
        sl = pl.ds(_off(t, D // NAUX), D // NAUX)
        return pltpu.make_async_copy(wo_h.at[:, sl], wo_v.at[:, sl], sem_in.at[s_o + t])

    def cp_out(i, t):
        sl = rows(0, MA, i, MA)
        c0, c1 = OUT_SPLIT[t], OUT_SPLIT[t + 1]
        return pltpu.make_async_copy(out_v.at[sl, c0:c1], out_h.at[sl, c0:c1],
                                     sem_out.at[i * (len(OUT_SPLIT) - 1) + t])

    for n in range(len(PEEL_COPIES)):
        cp_peel(n).start()

    def issue(c, carry):
        cp_g(c).start(); cp_u(c).start(); cp_d(c).start()

        @pl.when(jnp.logical_and(c >= 2, c < 2 + NAUX))
        def _():
            cp_wq(c - 2).start(); cp_wo(c - 2).start()
        return carry

    lax.fori_loop(1, n1, issue, 0)
    cp_gw().start()
    cp_xr().start()

    lane8 = lax.broadcasted_iota(jnp.int32, (8, LANES), 1)
    odd = (lane8 & 1) == 1
    row8 = lax.broadcasted_iota(jnp.int32, (8, LANES), 0)

    def waits_for(never, toks, w):
        if not toks:
            return w
        top = [w[0:8, t * LANES:(t + 1) * LANES] for t in range(w.shape[1] // LANES)]
        top = [jnp.where(never, toks[t], v) if t in toks else v for t, v in enumerate(top)]
        return jnp.concatenate([jnp.concatenate(top, axis=1), w[8:, :]], axis=0)

    def tile(m, t):
        return m[0:8, t * LANES:(t + 1) * LANES]

    def permute_put(slot, u32):
        for g in range(2 * H):
            tmp_v[slot, pl.ds((g // 2) * PITCH + (g % 2) * 8, 8), :] = u32[g * 8:(g + 1) * 8, :]

    def permute_get(slot, dst, row0, col, never, toks):
        for n in range(2 * NCH * H // 8):
            je, a = divmod(n, H // 8)
            base = row0 + n * 8
            if not isinstance(base, int):
                base = pl.multiple_of(base, 8)
            val = tmp_v[slot, pl.ds(8 * (je % 2) + je // 2 + a * 8 * PITCH, 8, stride=PITCH), :]
            if toks:
                val = jnp.where(never, toks[n * len(toks) // (2 * NCH * H // 8)], val)
            dst[col, pl.ds(base, 8), :] = val

    def after(never, tok, u32):
        return jnp.concatenate(
            [jnp.concatenate([jnp.where(never, tok, u32[r:r + 8, c:c + LANES])
                              for c in range(0, u32.shape[1], LANES)], axis=1)
             for r in range(0, u32.shape[0], 8)], axis=0)

    def prep_wq_put(slot, u, never, tok):
        kb, sec = lax.div(u, 3), lax.rem(u, 3)
        raw = pk(wqkv_v[rows(0, LANES, kb, LANES), pl.ds(_off(sec, D), D)])
        u32 = pltpu.bitcast(bf(after(never, tok, raw)).T, U32)
        permute_put(slot, u32)
        tok = u32[56:64, :]
        for t in range(1, NCH):
            tok = tok | u32[t * 64 + 56:t * 64 + 64, :]
        return tok

    def prep_wq_get(slot, u, never, toks):
        permute_get(slot, wt_v, _off(lax.rem(u, 3), D // 2), lax.div(u, 3), never, toks)

    def prep_wo_put(slot, c, never, toks):
        n = D // len(toks)
        col = pl.ds(_off(c, LANES), LANES)
        permute_put(slot, jnp.concatenate(
            [after(never, tok, pk(wo_v[rows(i * n, n), col])) for i, tok in enumerate(toks)], axis=0))

    def qkv(xa):
        for sec in QKV_ORDER:
            dst, r0 = ((q_v, 0), (k_v, HALO), (v_v, HALO))[sec]
            w = jnp.concatenate([wt_v[kb, sec * (D // 2):(sec + 1) * (D // 2), :] for kb in range(NCH)], axis=1)
            res = _dot_nt(xa, bf(w))
            for j in range(NCH):
                dst[j, r0:r0 + MA, :] = res[:, j * LANES:(j + 1) * LANES]

    def attn8(r, row0, never, tok, gate):
        sc = jnp.where(never, tok, scale * (LOG2E if EXP2 else 1.0))
        q = [q_v[j, r:r + 8, :] * sc for j in range(NCH)]
        logits = []
        valid = {}
        for w in range(WIN):
            lo = HALO + r - DIL * w
            s = q[0] * k_v[0, lo:lo + 8, :]
            for j in range(1, NCH):
                s = s + q[j] * k_v[j, lo:lo + 8, :]
            s = s + pltpu.roll(s, 64, 1)
            s = s + jnp.where(odd, pltpu.roll(s, 1, 1), pltpu.roll(s, LANES - 1, 1))
            if r - DIL * w < 0:
                valid[w] = row8 + (row0 + r - DIL * w) >= 0
                s = jnp.where(valid[w], s, NEG * (LOG2E if EXP2 else 1.0))
            logits.append(s)
        m = logits[0]
        for w in range(1, WIN):
            m = jnp.maximum(m, logits[w])
        p = [(jnp.exp2 if EXP2 else jnp.exp)(l - m) for l in logits]
        den = p[0]
        for w in range(1, WIN):
            den = den + p[w]
        inv = pl.reciprocal(den, approx=True)
        inv = inv * (2.0 - den * inv) * gate
        p = [pw * inv for pw in p]
        pm = None
        for w in valid:
            t = jnp.where(valid[w], 0.0, p[w])
            pm = t if pm is None else pm + t
        outs = []
        for j in range(NCH):
            acc = p[0] * v_v[j, HALO + r:HALO + r + 8, :]
            for w in range(1, WIN):
                lo = HALO + r - DIL * w
                acc = acc + p[w] * v_v[j, lo:lo + 8, :]
            if pm is not None:
                acc = acc + pm * v_v[j, HALO:HALO + 1, :]
            outs.append(acc)
        return outs, pltpu.bitcast(inv, U32)

    def attn16(r, i, never, tok_g, tok_a, tok_b):
        row0 = i * MA
        xg = bf(after(never, pltpu.bitcast(tok_g, U32), pk(x_v[rows(r, 16, i, MA), :]))).astype(F32)
        z = jnp.sum(xg * gw_v[...].astype(F32).reshape(1, D), axis=-1, keepdims=True)
        th = 0.5 * jnp.tanh(jnp.broadcast_to(0.5 * z, (16, LANES)))
        gate = 0.5 + th
        og_v[r:r + 16, :] = 0.5 - th
        a, done_a = attn8(r, row0, never, tok_a, gate[0:8])
        b, done_b = attn8(r + 8, row0, never, tok_b, gate[8:16])
        for j in range(NCH):
            o_v[r // 2:r // 2 + 8, j * LANES:(j + 1) * LANES] = pltpu.bitcast(
                jnp.concatenate([a[j], b[j]], axis=0).astype(BF16), U32)
        return done_a, done_b

    def clear(j, carry):
        k_v[j, MA:MA + HALO, :] = jnp.zeros((HALO, LANES), F32)
        v_v[j, MA:MA + HALO, :] = jnp.zeros((HALO, LANES), F32)
        wqkv_v[rows(D, 16, j, 16), 0:D] = jnp.zeros((16 // PK, D), wqkv_v.dtype)
        wo_v[rows(0, LANES, j, LANES), D:] = jnp.zeros((LANES // PK, LANES), wo_v.dtype)
        return carry

    lax.fori_loop(0, NCH, clear, 0)

    parts = {}
    for waits, work in PEEL_STEPS:
        for n in waits:
            cp_peel(n).wait()
        for kind, r0, r1, c0, c1 in work:
            if kind in "gu":
                w_v = wg_v if kind == "g" else wu_v
                parts[kind, r0, c0] = (r1, c1, _dot(bf(pk(x_v[rows(r0, r1 - r0), :])), bf(pk(w_v[:, c0:c1]))))
            elif kind == "h":
                def gather(kd):
                    cols = []
                    for cc in sorted({k[2] for k in parts if k[0] == kd and c0 <= k[2] < c1}):
                        rs = sorted(k[1] for k in parts if k[0] == kd and k[2] == cc)
                        cols.append(jnp.concatenate([parts[kd, r, cc][2] for r in rs], axis=0))
                    return jnp.concatenate(cols, axis=1)
                parts["h", 0, c0] = (r1, c1, (jnp.maximum(gather("g"), 0.0) * gather("u")).astype(BF16))
            else:
                h = jnp.concatenate([parts[k][2] for k in sorted(parts) if k[0] == "h" and c0 <= k[2] < c1], axis=1)
                r = _dot(h, bf(pk(wd_v[rows(c0, c1 - c0), :])))
                if c0 == 0:
                    b_v[0:R1, :] = r
                else:
                    b_v[0:R1, :] += r

    def p1_body(c, carry):
        aux = jnp.logical_and(c >= 2, c < 2 + NAUX)
        ta = jnp.clip(c - 2, 0, NAUX - 1)
        cp_g(c).wait(); cp_u(c).wait(); cp_d(c).wait()
        pl.when(aux)(cp_wq(ta).wait)
        pl.when(aux)(cp_wo(ta).wait)
        uq = [UQ * c + t - Q0 for t in range(UQ)]
        uo = [UO * c + t - O0 for t in range(UO)]
        uq = [jnp.where(jnp.logical_and(u >= 0, u < NU), u, NU) for u in uq]
        uo = [jnp.where(jnp.logical_and(u >= 0, u < NCH), u, NCH) for u in uo]
        off = _off(c, FC1)
        xv = bf(pk(x_v[rows(0, R1), :]))
        never = row8 + c < 0
        nt = FC1 // LANES
        res = []
        done = {}
        for m in range(2 * nt):
            w_v = wg_v if m < nt else wu_v
            w = pk(w_v[:, pl.ds(pl.multiple_of(off + (m % nt) * LANES, LANES), LANES)])
            r = _dot(xv, bf(waits_for(never, {0: done[m]} if m in done else None, w)))
            res.append(r)
            if m < UQ:
                done[m + P1_LAG] = prep_wq_put(m, uq[m], never, pltpu.bitcast(r[0:8, :], U32))
            if 0 <= m - P1_LAG < UQ:
                toks = [pltpu.bitcast(r[rr:rr + 8, :], U32) for rr in range(0, R1, P1_GET_STEP)] if P1_GET_STEP else None
                prep_wq_get(m - P1_LAG, uq[m - P1_LAG], never, toks)
        g = jnp.concatenate(res[:nt], axis=1)
        u = jnp.concatenate(res[nt:], axis=1)
        h = (jnp.maximum(g, 0.0) * u).astype(BF16)
        r = _dot(h, bf(pk(wd_v[rows(0, FC1, c, FC1), :])))
        b_v[0:R1, :] += r
        for t in range(UO):
            toks = [pltpu.bitcast(r[rr:rr + 8, tt * LANES:(tt + 1) * LANES], U32)
                    for tt in WO_TILES[t] for rr in range(0, R1, R1 // 4)]
            prep_wo_put(UQ + t, uo[t], never, toks)
            tt = WO_TILES[t][-1] + 1
            toks = ([pltpu.bitcast(r[rr:rr + 8, tt * LANES:(tt + 1) * LANES], U32)
                     for rr in range(0, R1, P1_GET_STEP)] if P1_GET_STEP else None)
            permute_get(UQ + t, wop_v, 0, uo[t], never, toks)
        return carry

    lax.fori_loop(1, n1, p1_body, 0)
    cp_gw().wait()
    cp_xr().wait()

    def p2_body(i, carry):
        ra = pl.multiple_of(i * MA, MA)
        rf = pl.multiple_of(R1 + i * MF, 16)
        k_v[:, 0:HALO, :] = k_v[:, MA:MA + HALO, :]
        v_v[:, 0:HALO, :] = v_v[:, MA:MA + HALO, :]
        never = row8 + i < 0
        groups = iter(range(0, MA, 16))

        def attn_group(m, k):
            r = next(groups, None)
            if r is None:
                return None
            return dict(zip(DEADLINES[k], attn16(r, i, never, *(tile(m, t) for t in TOKS[k]))))

        dl = None
        if QKV_AFTER < 0:
            qkv(bf(pk(x_v[rows(0, MA, i, MA), :])))
        for c in range(n2):
            off = c * FC2
            xv = bf(pk(x_v[rows(R1, MF, i, MF), :]))
            g = _dot(xv, bf(waits_for(never, dl, pk(wg_v[:, off:off + FC2]))))
            dl = attn_group(g, 0) if c > QKV_AFTER else None
            u = _dot(xv, bf(waits_for(never, dl, pk(wu_v[:, off:off + FC2]))))
            dl = attn_group(u, 1) if c > QKV_AFTER else None
            h = (jnp.maximum(g, 0.0) * u).astype(BF16)
            r = _dot(h, bf(waits_for(never, dl, pk(wd_v[rows(off, FC2), :]))))
            if c == 0:
                b_v[pl.ds(rf, MF), :] = r
            else:
                b_v[pl.ds(rf, MF), :] += r
            if c == QKV_AFTER:
                qkv(bf(pk(x_v[rows(0, MA, i, MA), :])))
            dl = attn_group(r, 2) if c > QKV_AFTER else None
        for t in range(len(OUT_SPLIT) - 1):
            c0, c1 = OUT_SPLIT[t], OUT_SPLIT[t + 1]
            tiles = range(c0 // LANES, c1 // LANES)
            a = _dot(bf(o_v[...]), bf(jnp.concatenate([wop_v[c] for c in tiles], axis=1)))
            og = jnp.concatenate([og_v[...]] * len(tiles), axis=1)
            res = (a + og * b_v[pl.ds(ra, MA), c0:c1]).astype(BF16)
            out_v[rows(0, MA, i, MA), c0:c1] = pltpu.bitcast(res, U32) if NATIVE else res
            cp_out(i, t).start()
        return carry

    lax.fori_loop(0, NIT, p2_body, 0)
    for i in range(NIT):
        for t in range(len(OUT_SPLIT) - 1):
            cp_out(i, t).wait()


@jax.jit
def pallas_gated_mix__sliding_local_dilated__glu_gated_reglu__prompt_kernel(
    A_x: jax.Array,
    A_wqkv: jax.Array,
    A_wo: jax.Array,
    B_x: jax.Array,
    B_W_gate: jax.Array,
    B_W_up: jax.Array,
    B_W_down: jax.Array,
    gate_w: jax.Array,
):
    B, S, D = A_x.shape
    assert B == 1
    F = B_W_gate.shape[1]
    NCH = D // LANES
    MA = S // NIT
    n1 = F // FC1
    n_in = len(PEEL_COPIES) + 2 + 3 * (n1 - 1) + 2 * NAUX

    def kernel(*refs):
        def once(_, c):
            _kernel(*refs, S=S, D=D, F=F)
            return c

        lax.fori_loop(0, pl.program_id(0) + 1, once, 0)

    def cbuf(r, c):
        return pltpu.VMEM((r // 2, c), U32) if NATIVE else pltpu.VMEM((r, c), BF16)

    any_spec = pl.BlockSpec(memory_space=pl.ANY)
    return pl.pallas_call(
        kernel,
        grid=(1,),
        in_specs=[any_spec] * 7,
        out_specs=any_spec,
        out_shape=jax.ShapeDtypeStruct((B, S, D), A_x.dtype),
        scratch_shapes=[
            cbuf(S, D),
            cbuf(D + LANES, 3 * D),
            cbuf(D, D + LANES),
            cbuf(D, F),
            cbuf(D, F),
            cbuf(F, D),
            pltpu.VMEM((D,), BF16),
            pltpu.VMEM((NCH + 1, 3 * D // 2, LANES), U32),
            pltpu.VMEM((NCH + 1, D // 2, LANES), U32),
            pltpu.VMEM((UQ + UO, TMP_ROWS, LANES), U32),
            pltpu.VMEM((S, D), F32),
            pltpu.VMEM((NCH, MA, LANES), F32),
            pltpu.VMEM((NCH, HALO + MA + KV_PAD, LANES), F32),
            pltpu.VMEM((NCH, HALO + MA + KV_PAD, LANES), F32),
            pltpu.VMEM((MA // 2, D), U32),
            pltpu.VMEM((MA, LANES), F32),
            cbuf(S, D),
            pltpu.SemaphoreType.DMA((n_in,)),
            pltpu.SemaphoreType.DMA((NIT * (len(OUT_SPLIT) - 1),)),
        ],
        compiler_params=pltpu.CompilerParams(
            vmem_limit_bytes=100 * 1024 * 1024,
            disable_semaphore_checks=True,
            disable_bounds_checks=True,
        ),
    )(A_x, A_wqkv, A_wo, B_W_gate, B_W_up, B_W_down, gate_w)
```

```python
import jax
import jax.numpy as jnp
from jax import lax
import jax.experimental.pallas as pl
import jax.experimental.pallas.tpu as pltpu

H = 32
WIN = 8
DIL = 2
HALO = 16
LANES = 128
NEG = -1e9
LOG2E = 1.4426950408889634

R1 = 512
FC1 = 512
FC2 = 512
NIT = 8
PITCH = 17

TOKS = ((0, 1, 3), (0, 1, 3), (0, 2, 6))
DEADLINES = ((0, 2), (0, 4), (0, 2))
UQ = 5
UO = 2
NAUX = 4
P1_LAG = 2
K_ORDER = (3, 2, 1, 0, 7, 6, 5, 4)
NATIVE = False
EXP2 = True
QKV_ORDER = (1, 0, 2)
QKV_AFTER = 0
P1_GET_STEP = 8
OUT_SPLIT = (0, 1024)
WO_TILES = ((0, 1), (3, 4))
TMP_ROWS = 552
KV_PAD = 0

PEEL_COPIES = (("x", 0, 128), ("g", 0, 128), ("x", 128, 256), ("g", 128, 256), ("x", 256, 512),
               ("u", 0, 256), ("g", 256, 512), ("u", 256, 512), ("d", 0, 512))
PEEL_STEPS = (
    ((0, 1), (("g", 0, 128, 0, 128),)),
    ((2,), (("g", 128, 256, 0, 128),)),
    ((3,), (("g", 0, 256, 128, 256),)),
    ((4,), (("g", 256, 512, 0, 128), ("g", 256, 512, 128, 256))),
    ((5,), (("u", 0, 512, 0, 256), ("h", 0, 512, 0, 256))),
    ((6, 7), (("g", 0, 512, 256, 512), ("u", 0, 512, 256, 512), ("h", 0, 512, 256, 512))),
    ((8,), (("d", 0, 512, 0, 512),)),
)

F32 = jnp.float32
BF16 = jnp.bfloat16
U32 = jnp.uint32


def _dot(a, b):
    return jnp.dot(a, b, preferred_element_type=F32)


def _dot_nt(a, b):
    return lax.dot_general(a, b, (((1,), (1,)), ((), ())), preferred_element_type=F32)


def _kernel(x_hbm, wqkv_hbm, wo_hbm, wg_hbm, wu_hbm, wd_hbm, gw_hbm, out_hbm,
            x_v, wqkv_v, wo_v, wg_v, wu_v, wd_v, gw_v,
            wt_v, wop_v, tmp_v, b_v, q_v, k_v, v_v, o_v, og_v, out_v,
            sem_in, sem_out, *, S, D, F):
    NCH = D // LANES
    DH = D // H
    scale = DH ** -0.5
    n1 = F // FC1
    n2 = F // FC2
    MF = (S - R1) // NIT
    MA = S // NIT
    NU = 3 * NCH
    Q0 = 2 * UQ
    O0 = 2 * UO
    assert UQ * (n1 - 1) + UQ - 1 - Q0 >= NU - 1 and UO * (n1 - 1) + UO - 1 - O0 >= NCH - 1

    PK = 2 if NATIVE else 1
    hb = (lambda r: r.bitcast(U32)) if NATIVE else (lambda r: r)
    x_h = hb(x_hbm.at[0])
    out_h = hb(out_hbm.at[0])
    wqkv_h, wo_h, wg_h, wu_h, wd_h = (hb(r) for r in (wqkv_hbm, wo_hbm, wg_hbm, wu_hbm, wd_hbm))

    def _off(c, n):
        return c * n if isinstance(c, int) else pl.multiple_of(c * n, n)

    def rows(start, n, i=0, step=0):
        if isinstance(i, int):
            return pl.ds((start + i * step) // PK, n // PK)
        return pl.ds(pl.multiple_of(start // PK + i * (step // PK), 16 // PK), n // PK)

    def pk(v):
        return v if NATIVE else pltpu.bitcast(v, U32)

    def bf(v):
        return pltpu.bitcast(v, BF16)

    s_p = 0
    s_gw = len(PEEL_COPIES)
    s_xr = s_gw + 1
    s_w = s_xr + 1 - 3
    s_u = s_w + 3 * n1
    s_o = s_u + NAUX

    def cp_peel(n):
        kind, lo, hi = PEEL_COPIES[n]
        if kind == "x":
            sl = rows(lo, hi - lo)
            return pltpu.make_async_copy(x_h.at[sl, :], x_v.at[sl, :], sem_in.at[s_p + n])
        if kind == "d":
            sl = rows(lo, hi - lo)
            return pltpu.make_async_copy(wd_h.at[sl, :], wd_v.at[sl, :], sem_in.at[s_p + n])
        src, dst = (wg_h, wg_v) if kind == "g" else (wu_h, wu_v)
        sl = pl.ds(lo, hi - lo)
        return pltpu.make_async_copy(src.at[:, sl], dst.at[:, sl], sem_in.at[s_p + n])

    def cp_xr():
        sl = rows(R1, S - R1)
        return pltpu.make_async_copy(x_h.at[sl, :], x_v.at[sl, :], sem_in.at[s_xr])

    def cp_gw():
        return pltpu.make_async_copy(gw_hbm, gw_v, sem_in.at[s_gw])

    def cp_g(c):
        sl = pl.ds(_off(c, FC1), FC1)
        return pltpu.make_async_copy(wg_h.at[:, sl], wg_v.at[:, sl], sem_in.at[s_w + 3 * c])

    def cp_u(c):
        sl = pl.ds(_off(c, FC1), FC1)
        return pltpu.make_async_copy(wu_h.at[:, sl], wu_v.at[:, sl], sem_in.at[s_w + 3 * c + 1])

    def cp_d(c):
        sl = rows(0, FC1, c, FC1)
        return pltpu.make_async_copy(wd_h.at[sl, :], wd_v.at[sl, :], sem_in.at[s_w + 3 * c + 2])

    def cp_wq(t):
        sl = rows(0, D // NAUX, t, D // NAUX)
        return pltpu.make_async_copy(wqkv_h.at[sl, :], wqkv_v.at[sl, :], sem_in.at[s_u + t])

    def cp_wo(t):
        sl = pl.ds(_off(t, D // NAUX), D // NAUX)
        return pltpu.make_async_copy(wo_h.at[:, sl], wo_v.at[:, sl], sem_in.at[s_o + t])

    def cp_out(i, t):
        sl = rows(0, MA, i, MA)
        c0, c1 = OUT_SPLIT[t], OUT_SPLIT[t + 1]
        return pltpu.make_async_copy(out_v.at[sl, c0:c1], out_h.at[sl, c0:c1],
                                     sem_out.at[i * (len(OUT_SPLIT) - 1) + t])

    for n in range(len(PEEL_COPIES)):
        cp_peel(n).start()

    def issue(c, carry):
        cp_g(c).start(); cp_u(c).start(); cp_d(c).start()

        @pl.when(jnp.logical_and(c >= 2, c < 2 + NAUX))
        def _():
            cp_wq(c - 2).start(); cp_wo(c - 2).start()
        return carry

    lax.fori_loop(1, n1, issue, 0)
    cp_gw().start()
    cp_xr().start()

    lane8 = lax.broadcasted_iota(jnp.int32, (8, LANES), 1)
    odd = (lane8 & 1) == 1
    row8 = lax.broadcasted_iota(jnp.int32, (8, LANES), 0)

    def waits_for(never, toks, w):
        if not toks:
            return w
        top = [w[0:8, t * LANES:(t + 1) * LANES] for t in range(w.shape[1] // LANES)]
        top = [jnp.where(never, toks[t], v) if t in toks else v for t, v in enumerate(top)]
        return jnp.concatenate([jnp.concatenate(top, axis=1), w[8:, :]], axis=0)

    def tile(m, t):
        return m[0:8, t * LANES:(t + 1) * LANES]

    def permute_put(slot, u32):
        for g in range(2 * H):
            tmp_v[slot, pl.ds((g // 2) * PITCH + (g % 2) * 8, 8), :] = u32[g * 8:(g + 1) * 8, :]

    def permute_get(slot, dst, row0, col, never, toks):
        for n in range(2 * NCH * H // 8):
            je, a = divmod(n, H // 8)
            base = row0 + n * 8
            if not isinstance(base, int):
                base = pl.multiple_of(base, 8)
            val = tmp_v[slot, pl.ds(8 * (je % 2) + je // 2 + a * 8 * PITCH, 8, stride=PITCH), :]
            if toks:
                val = jnp.where(never, toks[n * len(toks) // (2 * NCH * H // 8)], val)
            dst[col, pl.ds(base, 8), :] = val

    def after(never, tok, u32):
        return jnp.concatenate(
            [jnp.concatenate([jnp.where(never, tok, u32[r:r + 8, c:c + LANES])
                              for c in range(0, u32.shape[1], LANES)], axis=1)
             for r in range(0, u32.shape[0], 8)], axis=0)

    def prep_wq_put(slot, u, never, tok):
        kb, sec = lax.div(u, 3), lax.rem(u, 3)
        raw = pk(wqkv_v[rows(0, LANES, kb, LANES), pl.ds(_off(sec, D), D)])
        u32 = pltpu.bitcast(bf(after(never, tok, raw)).T, U32)
        permute_put(slot, u32)
        tok = u32[56:64, :]
        for t in range(1, NCH):
            tok = tok | u32[t * 64 + 56:t * 64 + 64, :]
        return tok

    def prep_wq_get(slot, u, never, toks):
        permute_get(slot, wt_v, _off(lax.rem(u, 3), D // 2), lax.div(u, 3), never, toks)

    def prep_wo_put(slot, c, never, toks):
        n = D // len(toks)
        col = pl.ds(_off(c, LANES), LANES)
        permute_put(slot, jnp.concatenate(
            [after(never, tok, pk(wo_v[rows(i * n, n), col])) for i, tok in enumerate(toks)], axis=0))

    def qkv(xa):
        for sec in QKV_ORDER:
            dst, r0 = ((q_v, 0), (k_v, HALO), (v_v, HALO))[sec]
            w = jnp.concatenate([wt_v[kb, sec * (D // 2):(sec + 1) * (D // 2), :] for kb in range(NCH)], axis=1)
            res = _dot_nt(xa, bf(w))
            for j in range(NCH):
                dst[j, r0:r0 + MA, :] = res[:, j * LANES:(j + 1) * LANES]

    def attn8(r, row0, never, tok, gate):
        sc = jnp.where(never, tok, scale * (LOG2E if EXP2 else 1.0))
        q = [q_v[j, r:r + 8, :] * sc for j in range(NCH)]
        logits = []
        valid = {}
        for w in range(WIN):
            lo = HALO + r - DIL * w
            s = q[0] * k_v[0, lo:lo + 8, :]
            for j in range(1, NCH):
                s = s + q[j] * k_v[j, lo:lo + 8, :]
            s = s + pltpu.roll(s, 64, 1)
            s = s + jnp.where(odd, pltpu.roll(s, 1, 1), pltpu.roll(s, LANES - 1, 1))
            if r - DIL * w < 0:
                valid[w] = row8 + (row0 + r - DIL * w) >= 0
                s = jnp.where(valid[w], s, NEG * (LOG2E if EXP2 else 1.0))
            logits.append(s)
        m = logits[0]
        for w in range(1, WIN):
            m = jnp.maximum(m, logits[w])
        p = [(jnp.exp2 if EXP2 else jnp.exp)(l - m) for l in logits]
        den = p[0]
        for w in range(1, WIN):
            den = den + p[w]
        inv = pl.reciprocal(den, approx=True)
        inv = inv * (2.0 - den * inv) * gate
        p = [pw * inv for pw in p]
        pm = None
        for w in valid:
            t = jnp.where(valid[w], 0.0, p[w])
            pm = t if pm is None else pm + t
        outs = []
        for j in range(NCH):
            acc = p[0] * v_v[j, HALO + r:HALO + r + 8, :]
            for w in range(1, WIN):
                lo = HALO + r - DIL * w
                acc = acc + p[w] * v_v[j, lo:lo + 8, :]
            if pm is not None:
                acc = acc + pm * v_v[j, HALO:HALO + 1, :]
            outs.append(acc)
        return outs, pltpu.bitcast(inv, U32)

    def attn16(r, i, never, tok_g, tok_a, tok_b):
        row0 = i * MA
        xg = bf(after(never, pltpu.bitcast(tok_g, U32), pk(x_v[rows(r, 16, i, MA), :]))).astype(F32)
        z = jnp.sum(xg * gw_v[...].astype(F32).reshape(1, D), axis=-1, keepdims=True)
        th = 0.5 * jnp.tanh(jnp.broadcast_to(0.5 * z, (16, LANES)))
        gate = 0.5 + th
        og_v[r:r + 16, :] = 0.5 - th
        a, done_a = attn8(r, row0, never, tok_a, gate[0:8])
        b, done_b = attn8(r + 8, row0, never, tok_b, gate[8:16])
        for j in range(NCH):
            o_v[r // 2:r // 2 + 8, j * LANES:(j + 1) * LANES] = pltpu.bitcast(
                jnp.concatenate([a[j], b[j]], axis=0).astype(BF16), U32)
        return done_a, done_b

    def clear(j, carry):
        k_v[j, MA:MA + HALO, :] = jnp.zeros((HALO, LANES), F32)
        v_v[j, MA:MA + HALO, :] = jnp.zeros((HALO, LANES), F32)
        wqkv_v[rows(D, 16, j, 16), 0:D] = jnp.zeros((16 // PK, D), wqkv_v.dtype)
        wo_v[rows(0, LANES, j, LANES), D:] = jnp.zeros((LANES // PK, LANES), wo_v.dtype)
        return carry

    lax.fori_loop(0, NCH, clear, 0)

    parts = {}
    for waits, work in PEEL_STEPS:
        for n in waits:
            cp_peel(n).wait()
        for kind, r0, r1, c0, c1 in work:
            if kind in "gu":
                w_v = wg_v if kind == "g" else wu_v
                parts[kind, r0, c0] = (r1, c1, _dot(bf(pk(x_v[rows(r0, r1 - r0), :])), bf(pk(w_v[:, c0:c1]))))
            elif kind == "h":
                def gather(kd):
                    cols = []
                    for cc in sorted({k[2] for k in parts if k[0] == kd and c0 <= k[2] < c1}):
                        rs = sorted(k[1] for k in parts if k[0] == kd and k[2] == cc)
                        cols.append(jnp.concatenate([parts[kd, r, cc][2] for r in rs], axis=0))
                    return jnp.concatenate(cols, axis=1)
                parts["h", 0, c0] = (r1, c1, (jnp.maximum(gather("g"), 0.0) * gather("u")).astype(BF16))
            else:
                h = jnp.concatenate([parts[k][2] for k in sorted(parts) if k[0] == "h" and c0 <= k[2] < c1], axis=1)
                r = _dot(h, bf(pk(wd_v[rows(c0, c1 - c0), :])))
                if c0 == 0:
                    b_v[0:R1, :] = r
                else:
                    b_v[0:R1, :] += r

    def p1_body(c, carry):
        aux = jnp.logical_and(c >= 2, c < 2 + NAUX)
        ta = jnp.clip(c - 2, 0, NAUX - 1)
        cp_g(c).wait(); cp_u(c).wait(); cp_d(c).wait()
        pl.when(aux)(cp_wq(ta).wait)
        pl.when(aux)(cp_wo(ta).wait)
        uq = [UQ * c + t - Q0 for t in range(UQ)]
        uo = [UO * c + t - O0 for t in range(UO)]
        uq = [jnp.where(jnp.logical_and(u >= 0, u < NU), u, NU) for u in uq]
        uo = [jnp.where(jnp.logical_and(u >= 0, u < NCH), u, NCH) for u in uo]
        off = _off(c, FC1)
        xv = bf(pk(x_v[rows(0, R1), :]))
        never = row8 + c < 0
        nt = FC1 // LANES
        res = []
        done = {}
        for m in range(2 * nt):
            w_v = wg_v if m < nt else wu_v
            w = pk(w_v[:, pl.ds(pl.multiple_of(off + (m % nt) * LANES, LANES), LANES)])
            r = _dot(xv, bf(waits_for(never, {0: done[m]} if m in done else None, w)))
            res.append(r)
            if m < UQ:
                done[m + P1_LAG] = prep_wq_put(m, uq[m], never, pltpu.bitcast(r[0:8, :], U32))
            if 0 <= m - P1_LAG < UQ:
                toks = [pltpu.bitcast(r[rr:rr + 8, :], U32) for rr in range(0, R1, P1_GET_STEP)] if P1_GET_STEP else None
                prep_wq_get(m - P1_LAG, uq[m - P1_LAG], never, toks)
        g = jnp.concatenate(res[:nt], axis=1)
        u = jnp.concatenate(res[nt:], axis=1)
        h = (jnp.maximum(g, 0.0) * u).astype(BF16)
        r = _dot(h, bf(pk(wd_v[rows(0, FC1, c, FC1), :])))
        b_v[0:R1, :] += r
        for t in range(UO):
            toks = [pltpu.bitcast(r[rr:rr + 8, tt * LANES:(tt + 1) * LANES], U32)
                    for tt in WO_TILES[t] for rr in range(0, R1, R1 // 4)]
            prep_wo_put(UQ + t, uo[t], never, toks)
            tt = WO_TILES[t][-1] + 1
            toks = ([pltpu.bitcast(r[rr:rr + 8, tt * LANES:(tt + 1) * LANES], U32)
                     for rr in range(0, R1, P1_GET_STEP)] if P1_GET_STEP else None)
            permute_get(UQ + t, wop_v, 0, uo[t], never, toks)
        return carry

    lax.fori_loop(1, n1, p1_body, 0)
    cp_gw().wait()
    cp_xr().wait()

    def p2_body(i, carry):
        ra = pl.multiple_of(i * MA, MA)
        rf = pl.multiple_of(R1 + i * MF, 16)
        k_v[:, 0:HALO, :] = k_v[:, MA:MA + HALO, :]
        v_v[:, 0:HALO, :] = v_v[:, MA:MA + HALO, :]
        never = row8 + i < 0
        groups = iter(range(0, MA, 16))

        def attn_group(m, k):
            r = next(groups, None)
            if r is None:
                return None
            return dict(zip(DEADLINES[k], attn16(r, i, never, *(tile(m, t) for t in TOKS[k]))))

        dl = None
        if QKV_AFTER < 0:
            qkv(bf(pk(x_v[rows(0, MA, i, MA), :])))
        for c in range(n2):
            off = c * FC2
            xv = bf(pk(x_v[rows(R1, MF, i, MF), :]))
            if c == 0 and K_ORDER:
                wk = pk(wg_v[:, off:off + FC2])
                g = _dot(jnp.concatenate([xv[:, t * LANES:(t + 1) * LANES] for t in K_ORDER], axis=1),
                         bf(jnp.concatenate([wk[t * 64:(t + 1) * 64, :] for t in K_ORDER], axis=0)))
            else:
                g = _dot(xv, bf(waits_for(never, dl, pk(wg_v[:, off:off + FC2]))))
            dl = attn_group(g, 0) if c > QKV_AFTER else None
            u = _dot(xv, bf(waits_for(never, dl, pk(wu_v[:, off:off + FC2]))))
            dl = attn_group(u, 1) if c > QKV_AFTER else None
            h = (jnp.maximum(g, 0.0) * u).astype(BF16)
            r = _dot(h, bf(waits_for(never, dl, pk(wd_v[rows(off, FC2), :]))))
            if c == 0:
                b_v[pl.ds(rf, MF), :] = r
            else:
                b_v[pl.ds(rf, MF), :] += r
            if c == QKV_AFTER:
                qkv(bf(pk(x_v[rows(0, MA, i, MA), :])))
            dl = attn_group(r, 2) if c > QKV_AFTER else None
        for t in range(len(OUT_SPLIT) - 1):
            c0, c1 = OUT_SPLIT[t], OUT_SPLIT[t + 1]
            tiles = range(c0 // LANES, c1 // LANES)
            a = _dot(bf(o_v[...]), bf(jnp.concatenate([wop_v[c] for c in tiles], axis=1)))
            og = jnp.concatenate([og_v[...]] * len(tiles), axis=1)
            res = (a + og * b_v[pl.ds(ra, MA), c0:c1]).astype(BF16)
            out_v[rows(0, MA, i, MA), c0:c1] = pltpu.bitcast(res, U32) if NATIVE else res
            cp_out(i, t).start()
        return carry

    lax.fori_loop(0, NIT, p2_body, 0)
    for i in range(NIT):
        for t in range(len(OUT_SPLIT) - 1):
            cp_out(i, t).wait()


@jax.jit
def pallas_gated_mix__sliding_local_dilated__glu_gated_reglu__prompt_kernel(
    A_x: jax.Array,
    A_wqkv: jax.Array,
    A_wo: jax.Array,
    B_x: jax.Array,
    B_W_gate: jax.Array,
    B_W_up: jax.Array,
    B_W_down: jax.Array,
    gate_w: jax.Array,
):
    B, S, D = A_x.shape
    assert B == 1
    F = B_W_gate.shape[1]
    NCH = D // LANES
    MA = S // NIT
    n1 = F // FC1
    n_in = len(PEEL_COPIES) + 2 + 3 * (n1 - 1) + 2 * NAUX

    def kernel(*refs):
        def once(_, c):
            _kernel(*refs, S=S, D=D, F=F)
            return c

        lax.fori_loop(0, pl.program_id(0) + 1, once, 0)

    def cbuf(r, c):
        return pltpu.VMEM((r // 2, c), U32) if NATIVE else pltpu.VMEM((r, c), BF16)

    any_spec = pl.BlockSpec(memory_space=pl.ANY)
    return pl.pallas_call(
        kernel,
        grid=(1,),
        in_specs=[any_spec] * 7,
        out_specs=any_spec,
        out_shape=jax.ShapeDtypeStruct((B, S, D), A_x.dtype),
        scratch_shapes=[
            cbuf(S, D),
            cbuf(D + LANES, 3 * D),
            cbuf(D, D + LANES),
            cbuf(D, F),
            cbuf(D, F),
            cbuf(F, D),
            pltpu.VMEM((D,), BF16),
            pltpu.VMEM((NCH + 1, 3 * D // 2, LANES), U32),
            pltpu.VMEM((NCH + 1, D // 2, LANES), U32),
            pltpu.VMEM((UQ + UO, TMP_ROWS, LANES), U32),
            pltpu.VMEM((S, D), F32),
            pltpu.VMEM((NCH, MA, LANES), F32),
            pltpu.VMEM((NCH, HALO + MA + KV_PAD, LANES), F32),
            pltpu.VMEM((NCH, HALO + MA + KV_PAD, LANES), F32),
            pltpu.VMEM((MA // 2, D), U32),
            pltpu.VMEM((MA, LANES), F32),
            cbuf(S, D),
            pltpu.SemaphoreType.DMA((n_in,)),
            pltpu.SemaphoreType.DMA((NIT * (len(OUT_SPLIT) - 1),)),
        ],
        compiler_params=pltpu.CompilerParams(
            vmem_limit_bytes=100 * 1024 * 1024,
            disable_semaphore_checks=True,
            disable_bounds_checks=True,
        ),
    )(A_x, A_wqkv, A_wo, B_W_gate, B_W_up, B_W_down, gate_w)
```

```python
import jax
import jax.numpy as jnp
from jax import lax
import jax.experimental.pallas as pl
import jax.experimental.pallas.tpu as pltpu

H = 32
WIN = 8
DIL = 2
NEG = -1e9

LANES = 128
LOG2E = 1.4426950408889634
HALO = 16

R1 = 512
FC = 512
NIT = 8
UQ = 5
UO = 2
NAUX = 4
PITCH = 17
TMP_ROWS = 552

TOKS = ((0, 1, 3), (0, 1, 3), (0, 2, 6))
DEADLINES = ((0, 2), (0, 4), (0, 2))
P1_LAG = 2
WO_TILES = ((0, 1), (3, 4))
K_ORDER = (3, 2, 1, 0, 7, 6, 5, 4)

PEEL_COPIES = (("x", 0, 128), ("g", 0, 128), ("x", 128, 256), ("g", 128, 256), ("x", 256, 512),
               ("u", 0, 256), ("g", 256, 512), ("u", 256, 512), ("d", 0, 512))
PEEL_STEPS = (
    ((0, 1), (("g", 0, 128, 0, 128),)),
    ((2,), (("g", 128, 256, 0, 128),)),
    ((3,), (("g", 0, 256, 128, 256),)),
    ((4,), (("g", 256, 512, 0, 128), ("g", 256, 512, 128, 256))),
    ((5,), (("u", 0, 512, 0, 256), ("h", 0, 512, 0, 256))),
    ((6, 7), (("g", 0, 512, 256, 512), ("u", 0, 512, 256, 512), ("h", 0, 512, 256, 512))),
    ((8,), (("d", 0, 512, 0, 512),)),
)

F32 = jnp.float32
BF16 = jnp.bfloat16
U32 = jnp.uint32


def _dot(a, b):
    return jnp.dot(a, b, preferred_element_type=F32)


def _dot_nt(a, b):
    return lax.dot_general(a, b, (((1,), (1,)), ((), ())), preferred_element_type=F32)


def _pk(v):
    return pltpu.bitcast(v, U32)


def _bf(v):
    return pltpu.bitcast(v, BF16)


def _ds(i, step, size=None, base=0, align=None):
    size = step if size is None else size
    start = base + i * step
    if not isinstance(start, int):
        start = pl.multiple_of(start, step if align is None else align)
    return pl.ds(start, size)


def _kernel(x_hbm, wqkv_hbm, wo_hbm, wg_hbm, wu_hbm, wd_hbm, gw_hbm, out_hbm,
            x_v, wqkv_v, wo_v, wg_v, wu_v, wd_v, gw_v,
            wt_v, wop_v, tmp_v, b_v, q_v, k_v, v_v, o_v, og_v, out_v,
            sem_in, sem_out, *, S, D, F):
    NCH = D // LANES
    scale = (D // H) ** -0.5
    nc = F // FC
    nt = FC // LANES
    MF = (S - R1) // NIT
    MA = S // NIT
    NU = 3 * NCH
    assert UQ * (nc - 2) >= NU and UO * (nc - 2) >= NCH and MA // 16 <= 3 * (nc - 1)

    s_gw = len(PEEL_COPIES)
    s_xr = s_gw + 1
    s_w = s_xr + 1 - 3
    s_q = s_w + 3 * nc
    s_o = s_q + NAUX

    def cp_rows(src, dst, sl, s):
        return pltpu.make_async_copy(src.at[sl, :], dst.at[sl, :], sem_in.at[s])

    def cp_cols(src, dst, sl, s):
        return pltpu.make_async_copy(src.at[:, sl], dst.at[:, sl], sem_in.at[s])

    def cp_peel(n):
        kind, lo, hi = PEEL_COPIES[n]
        cp, src, dst = {"x": (cp_rows, x_hbm.at[0], x_v), "g": (cp_cols, wg_hbm, wg_v),
                        "u": (cp_cols, wu_hbm, wu_v), "d": (cp_rows, wd_hbm, wd_v)}[kind]
        return cp(src, dst, pl.ds(lo, hi - lo), n)

    def cp_xr():
        return cp_rows(x_hbm.at[0], x_v, pl.ds(R1, S - R1), s_xr)

    def cp_gw():
        return pltpu.make_async_copy(gw_hbm, gw_v, sem_in.at[s_gw])

    def cp_g(c):
        return cp_cols(wg_hbm, wg_v, _ds(c, FC), s_w + 3 * c)

    def cp_u(c):
        return cp_cols(wu_hbm, wu_v, _ds(c, FC), s_w + 3 * c + 1)

    def cp_d(c):
        return cp_rows(wd_hbm, wd_v, _ds(c, FC), s_w + 3 * c + 2)

    def cp_wq(t):
        return cp_rows(wqkv_hbm, wqkv_v, _ds(t, D // NAUX), s_q + t)

    def cp_wo(t):
        return cp_cols(wo_hbm, wo_v, _ds(t, D // NAUX), s_o + t)

    def cp_out(i):
        sl = _ds(i, MA)
        return pltpu.make_async_copy(out_v.at[sl, :], out_hbm.at[0, sl, :], sem_out.at[i])

    for n in range(len(PEEL_COPIES)):
        cp_peel(n).start()

    def issue(c, carry):
        cp_g(c).start(); cp_u(c).start(); cp_d(c).start()

        @pl.when(jnp.logical_and(c >= 2, c < 2 + NAUX))
        def _():
            cp_wq(c - 2).start(); cp_wo(c - 2).start()
        return carry

    lax.fori_loop(1, nc, issue, 0)
    cp_gw().start()
    cp_xr().start()

    lane8 = lax.broadcasted_iota(jnp.int32, (8, LANES), 1)
    odd = (lane8 & 1) == 1
    row8 = lax.broadcasted_iota(jnp.int32, (8, LANES), 0)

    def tile(m, t, r=0):
        return m[r:r + 8, t * LANES:(t + 1) * LANES]

    def after(never, tok, u32):
        return jnp.concatenate(
            [jnp.concatenate([jnp.where(never, tok, tile(u32, t, r))
                              for t in range(u32.shape[1] // LANES)], axis=1)
             for r in range(0, u32.shape[0], 8)], axis=0)

    def waits_for(never, toks, w):
        if not toks:
            return w
        w = _pk(w)
        top = [jnp.where(never, toks[t], tile(w, t)) if t in toks else tile(w, t)
               for t in range(w.shape[1] // LANES)]
        return _bf(jnp.concatenate([jnp.concatenate(top, axis=1), w[8:, :]], axis=0))

    def permute_put(slot, u32):
        for g in range(2 * H):
            tmp_v[slot, pl.ds((g // 2) * PITCH + (g % 2) * 8, 8), :] = u32[g * 8:(g + 1) * 8, :]

    def permute_get(slot, dst, col, sec, never, toks):
        for n in range(D // 16):
            je, a = divmod(n, H // 8)
            val = tmp_v[slot, pl.ds(8 * (je % 2) + je // 2 + a * 8 * PITCH, 8, stride=PITCH), :]
            dst[col, _ds(sec, D // 2, 8, n * 8, 8), :] = jnp.where(never, toks[n], val)

    def wq_put(slot, kb, sec, never, tok):
        raw = _pk(wqkv_v[_ds(kb, LANES), _ds(sec, D)])
        u32 = _pk(_bf(after(never, tok, raw)).T)
        permute_put(slot, u32)
        done = u32[56:64, :]
        for t in range(1, NCH):
            done = done | u32[t * 64 + 56:t * 64 + 64, :]
        return done

    def wo_put(slot, c, never, toks):
        n = D // len(toks)
        permute_put(slot, jnp.concatenate(
            [after(never, tok, _pk(wo_v[i * n:(i + 1) * n, _ds(c, LANES)]))
             for i, tok in enumerate(toks)], axis=0))

    def qkv(xa):
        for sec, dst, r0 in ((1, k_v, HALO), (0, q_v, 0), (2, v_v, HALO)):
            w = jnp.concatenate([wt_v[kb, sec * (D // 2):(sec + 1) * (D // 2), :] for kb in range(NCH)],
                                axis=1)
            res = _dot_nt(xa, _bf(w))
            for j in range(NCH):
                dst[j, r0:r0 + MA, :] = res[:, j * LANES:(j + 1) * LANES]

    def attn8(r, row0, never, tok, gate):
        sc = jnp.where(never, tok, scale * LOG2E)
        q = [q_v[j, r:r + 8, :] * sc for j in range(NCH)]
        logits = []
        valid = {}
        for w in range(WIN):
            lo = HALO + r - DIL * w
            s = q[0] * k_v[0, lo:lo + 8, :]
            for j in range(1, NCH):
                s = s + q[j] * k_v[j, lo:lo + 8, :]
            s = s + pltpu.roll(s, 64, 1)
            s = s + jnp.where(odd, pltpu.roll(s, 1, 1), pltpu.roll(s, LANES - 1, 1))
            if r - DIL * w < 0:
                valid[w] = row8 + (row0 + r - DIL * w) >= 0
                s = jnp.where(valid[w], s, NEG * LOG2E)
            logits.append(s)
        m = logits[0]
        for w in range(1, WIN):
            m = jnp.maximum(m, logits[w])
        p = [jnp.exp2(l - m) for l in logits]
        den = p[0]
        for w in range(1, WIN):
            den = den + p[w]
        inv = pl.reciprocal(den, approx=True)
        inv = inv * (2.0 - den * inv) * gate
        p = [pw * inv for pw in p]
        pm = None
        for w in valid:
            t = jnp.where(valid[w], 0.0, p[w])
            pm = t if pm is None else pm + t
        outs = []
        for j in range(NCH):
            acc = p[0] * v_v[j, HALO + r:HALO + r + 8, :]
            for w in range(1, WIN):
                lo = HALO + r - DIL * w
                acc = acc + p[w] * v_v[j, lo:lo + 8, :]
            if pm is not None:
                acc = acc + pm * v_v[j, HALO:HALO + 1, :]
            outs.append(acc)
        return outs, pltpu.bitcast(inv, U32)

    def attn16(r, i, never, tok_g, tok_a, tok_b):
        xg = _pk(x_v[_ds(i, MA, 16, r, 16), :])
        xg = _bf(after(never, pltpu.bitcast(tok_g, U32), xg)).astype(F32)
        z = jnp.sum(xg * gw_v[...].astype(F32).reshape(1, D), axis=-1, keepdims=True)
        th = 0.5 * jnp.tanh(jnp.broadcast_to(0.5 * z, (16, LANES)))
        gate = 0.5 + th
        og_v[r:r + 16, :] = 0.5 - th
        a, done_a = attn8(r, i * MA, never, tok_a, gate[0:8])
        b, done_b = attn8(r + 8, i * MA, never, tok_b, gate[8:16])
        for j in range(NCH):
            o_v[r // 2:r // 2 + 8, j * LANES:(j + 1) * LANES] = _pk(
                jnp.concatenate([a[j], b[j]], axis=0).astype(BF16))
        return done_a, done_b

    def clear(j, carry):
        k_v[j, MA:MA + HALO, :] = jnp.zeros((HALO, LANES), F32)
        v_v[j, MA:MA + HALO, :] = jnp.zeros((HALO, LANES), F32)
        wqkv_v[_ds(j, 16, base=D), 0:D] = jnp.zeros((16, D), BF16)
        wo_v[_ds(j, LANES), D:] = jnp.zeros((LANES, LANES), BF16)
        return carry

    lax.fori_loop(0, NCH, clear, 0)

    parts = {}

    def gather(kind, c0, c1):
        cols = []
        for cc in sorted({k[2] for k in parts if k[0] == kind and c0 <= k[2] < c1}):
            rs = sorted(k[1] for k in parts if k[0] == kind and k[2] == cc)
            cols.append(jnp.concatenate([parts[kind, r, cc] for r in rs], axis=0))
        return jnp.concatenate(cols, axis=1)

    for waits, work in PEEL_STEPS:
        for n in waits:
            cp_peel(n).wait()
        for kind, r0, r1, c0, c1 in work:
            if kind in "gu":
                parts[kind, r0, c0] = _dot(x_v[r0:r1, :], (wg_v if kind == "g" else wu_v)[:, c0:c1])
            elif kind == "h":
                parts[kind, r0, c0] = (jnp.maximum(gather("g", c0, c1), 0.0) * gather("u", c0, c1)).astype(BF16)
            else:
                b_v[0:R1, :] = _dot(gather("h", c0, c1), wd_v[c0:c1, :])

    def p1_body(c, carry):
        aux = jnp.logical_and(c >= 2, c < 2 + NAUX)
        ta = jnp.clip(c - 2, 0, NAUX - 1)
        cp_g(c).wait(); cp_u(c).wait(); cp_d(c).wait()
        pl.when(aux)(cp_wq(ta).wait)
        pl.when(aux)(cp_wo(ta).wait)
        uq = [UQ * (c - 2) + t for t in range(UQ)]
        uo = [UO * (c - 2) + t for t in range(UO)]
        uq = [jnp.where(jnp.logical_and(u >= 0, u < NU), u, NU) for u in uq]
        uo = [jnp.where(jnp.logical_and(u >= 0, u < NCH), u, NCH) for u in uo]
        uq = [(lax.div(u, 3), lax.rem(u, 3)) for u in uq]
        xv = x_v[0:R1, :]
        never = row8 + c < 0
        res = []
        done = {}
        for m in range(2 * nt):
            w = (wg_v if m < nt else wu_v)[:, _ds(c, FC, LANES, (m % nt) * LANES, LANES)]
            r = _dot(xv, waits_for(never, done.get(m), w))
            res.append(r)
            if m < UQ:
                done[m + P1_LAG] = {0: wq_put(m, *uq[m], never, pltpu.bitcast(tile(r, 0), U32))}
            if 0 <= m - P1_LAG < UQ:
                toks = [pltpu.bitcast(tile(r, 0, rr), U32) for rr in range(0, R1, 8)]
                permute_get(m - P1_LAG, wt_v, *uq[m - P1_LAG], never, toks)
        g = jnp.concatenate(res[:nt], axis=1)
        u = jnp.concatenate(res[nt:], axis=1)
        r = _dot((jnp.maximum(g, 0.0) * u).astype(BF16), wd_v[_ds(c, FC), :])
        b_v[0:R1, :] += r
        for t in range(UO):
            toks = [pltpu.bitcast(tile(r, tt, rr), U32) for tt in WO_TILES[t] for rr in range(0, R1, R1 // 4)]
            wo_put(UQ + t, uo[t], never, toks)
            toks = [pltpu.bitcast(tile(r, WO_TILES[t][-1] + 1, rr), U32) for rr in range(0, R1, 8)]
            permute_get(UQ + t, wop_v, uo[t], 0, never, toks)
        return carry

    lax.fori_loop(1, nc, p1_body, 0)
    cp_gw().wait()
    cp_xr().wait()

    def p2_body(i, carry):
        ra = _ds(i, MA)
        rf = _ds(i, MF, base=R1, align=16)
        k_v[:, 0:HALO, :] = k_v[:, MA:MA + HALO, :]
        v_v[:, 0:HALO, :] = v_v[:, MA:MA + HALO, :]
        never = row8 + i < 0
        groups = iter(range(0, MA, 16))

        def attn_group(m, k):
            r = next(groups, None)
            if r is None:
                return None
            return dict(zip(DEADLINES[k], attn16(r, i, never, *(tile(m, t) for t in TOKS[k]))))

        dl = None
        for c in range(nc):
            cols = slice(c * FC, (c + 1) * FC)
            xv = x_v[rf, :]
            if c == 0:
                wk = wg_v[:, cols]
                g = _dot(jnp.concatenate([xv[:, t * LANES:(t + 1) * LANES] for t in K_ORDER], axis=1),
                         jnp.concatenate([wk[t * LANES:(t + 1) * LANES, :] for t in K_ORDER], axis=0))
                h = (jnp.maximum(g, 0.0) * _dot(xv, wu_v[:, cols])).astype(BF16)
                b_v[rf, :] = _dot(h, wd_v[cols, :])
                qkv(x_v[ra, :])
                continue
            g = _dot(xv, waits_for(never, dl, wg_v[:, cols]))
            dl = attn_group(g, 0)
            u = _dot(xv, waits_for(never, dl, wu_v[:, cols]))
            dl = attn_group(u, 1)
            h = (jnp.maximum(g, 0.0) * u).astype(BF16)
            r = _dot(h, waits_for(never, dl, wd_v[cols, :]))
            b_v[rf, :] += r
            dl = attn_group(r, 2)
        a = _dot(_bf(o_v[...]), _bf(jnp.concatenate([wop_v[c] for c in range(NCH)], axis=1)))
        og = jnp.concatenate([og_v[...]] * NCH, axis=1)
        out_v[ra, :] = (a + og * b_v[ra, :]).astype(BF16)
        cp_out(i).start()
        return carry

    lax.fori_loop(0, NIT, p2_body, 0)
    for i in range(NIT):
        cp_out(i).wait()


@jax.jit
def pallas_gated_mix__sliding_local_dilated__glu_gated_reglu__prompt_kernel(
    A_x: jax.Array,
    A_wqkv: jax.Array,
    A_wo: jax.Array,
    B_x: jax.Array,
    B_W_gate: jax.Array,
    B_W_up: jax.Array,
    B_W_down: jax.Array,
    gate_w: jax.Array,
):
    B, S, D = A_x.shape
    assert B == 1
    F = B_W_gate.shape[1]
    NCH = D // LANES
    MA = S // NIT
    n_in = len(PEEL_COPIES) + 2 + 3 * (F // FC - 1) + 2 * NAUX

    def kernel(*refs):
        def once(_, c):
            _kernel(*refs, S=S, D=D, F=F)
            return c

        lax.fori_loop(0, pl.program_id(0) + 1, once, 0)

    any_spec = pl.BlockSpec(memory_space=pl.ANY)
    return pl.pallas_call(
        kernel,
        grid=(1,),
        in_specs=[any_spec] * 7,
        out_specs=any_spec,
        out_shape=jax.ShapeDtypeStruct((B, S, D), A_x.dtype),
        scratch_shapes=[
            pltpu.VMEM((S, D), BF16),
            pltpu.VMEM((D + LANES, 3 * D), BF16),
            pltpu.VMEM((D, D + LANES), BF16),
            pltpu.VMEM((D, F), BF16),
            pltpu.VMEM((D, F), BF16),
            pltpu.VMEM((F, D), BF16),
            pltpu.VMEM((D,), BF16),
            pltpu.VMEM((NCH + 1, 3 * D // 2, LANES), U32),
            pltpu.VMEM((NCH + 1, D // 2, LANES), U32),
            pltpu.VMEM((UQ + UO, TMP_ROWS, LANES), U32),
            pltpu.VMEM((S, D), F32),
            pltpu.VMEM((NCH, MA, LANES), F32),
            pltpu.VMEM((NCH, HALO + MA, LANES), F32),
            pltpu.VMEM((NCH, HALO + MA, LANES), F32),
            pltpu.VMEM((MA // 2, D), U32),
            pltpu.VMEM((MA, LANES), F32),
            pltpu.VMEM((S, D), BF16),
            pltpu.SemaphoreType.DMA((n_in,)),
            pltpu.SemaphoreType.DMA((NIT,)),
        ],
        compiler_params=pltpu.CompilerParams(
            vmem_limit_bytes=100 * 1024 * 1024,
            disable_semaphore_checks=True,
            disable_bounds_checks=True,
        ),
    )(A_x, A_wqkv, A_wo, B_W_gate, B_W_up, B_W_down, gate_w)
```

```python
import jax
import jax.numpy as jnp
from jax import lax
import jax.experimental.pallas as pl
import jax.experimental.pallas.tpu as pltpu

H = 32
WIN = 8
DIL = 2
NEG = -1e9

LANES = 128
LOG2E = 1.4426950408889634
HALO = 16

R1 = 512
FC = 512
NIT = 8
UQ = 5
UO = 2
NAUX = 4
PITCH = 17
TMP_ROWS = 552

TOKS = ((0, 1, 3), (0, 1, 3), (0, 2, 6))
DEADLINES = ((0, 2), (0, 4), (0, 2))
P1_LAG = 2
WO_TILES = ((0, 1), (3, 4))
K_ORDER = (3, 2, 1, 0, 7, 6, 5, 4)

PEEL_COPIES = (("x", 0, 256, 0, 512), ("g", 0, 512, 0, 256), ("x", 256, 512, 0, 512),
               ("g", 0, 512, 256, 512), ("x", 0, 512, 512, 1024), ("g", 512, 1024, 0, 256),
               ("g", 512, 1024, 256, 512), ("u", 0, 1024, 0, 256), ("u", 0, 1024, 256, 512),
               ("d", 0, 512, 0, 1024))
PEEL_STEPS = (
    ((0, 1), (("g", 0, 256, 0, 256, 0, 512),)),
    ((2,), (("g", 256, 512, 0, 256, 0, 512),)),
    ((3,), (("g", 0, 512, 256, 512, 0, 512),)),
    ((4, 5), (("g", 0, 512, 0, 256, 512, 1024),)),
    ((6,), (("g", 0, 512, 256, 512, 512, 1024),)),
    ((7,), (("u", 0, 512, 0, 256, 0, 1024), ("h", 0, 512, 0, 256, 0, 0))),
    ((8, 9), (("u", 0, 512, 256, 512, 0, 1024), ("h", 0, 512, 256, 512, 0, 0), ("d", 0, 512, 0, 512, 0, 0))),
)

F32 = jnp.float32
BF16 = jnp.bfloat16
U32 = jnp.uint32


def _dot(a, b):
    return jnp.dot(a, b, preferred_element_type=F32)


def _dot_nt(a, b):
    return lax.dot_general(a, b, (((1,), (1,)), ((), ())), preferred_element_type=F32)


def _pk(v):
    return pltpu.bitcast(v, U32)


def _bf(v):
    return pltpu.bitcast(v, BF16)


def _ds(i, step, size=None, base=0, align=None):
    size = step if size is None else size
    start = base + i * step
    if not isinstance(start, int):
        start = pl.multiple_of(start, step if align is None else align)
    return pl.ds(start, size)


def _kernel(x_hbm, wqkv_hbm, wo_hbm, wg_hbm, wu_hbm, wd_hbm, gw_hbm, out_hbm,
            x_v, wqkv_v, wo_v, wg_v, wu_v, wd_v, gw_v,
            wt_v, wop_v, tmp_v, b_v, q_v, k_v, v_v, o_v, og_v, out_v,
            sem_in, sem_out, *, S, D, F):
    NCH = D // LANES
    scale = (D // H) ** -0.5
    nc = F // FC
    nt = FC // LANES
    MF = (S - R1) // NIT
    MA = S // NIT
    NU = 3 * NCH
    assert UQ * (nc - 2) >= NU and UO * (nc - 2) >= NCH and MA // 16 <= 3 * (nc - 1)

    s_gw = len(PEEL_COPIES)
    s_xr = s_gw + 1
    s_w = s_xr + 1 - 3
    s_q = s_w + 3 * nc
    s_o = s_q + NAUX

    def cp_rows(src, dst, sl, s):
        return pltpu.make_async_copy(src.at[sl, :], dst.at[sl, :], sem_in.at[s])

    def cp_cols(src, dst, sl, s):
        return pltpu.make_async_copy(src.at[:, sl], dst.at[:, sl], sem_in.at[s])

    def cp_peel(n):
        kind, r0, r1, c0, c1 = PEEL_COPIES[n]
        src, dst = {"x": (x_hbm.at[0], x_v), "g": (wg_hbm, wg_v), "u": (wu_hbm, wu_v), "d": (wd_hbm, wd_v)}[kind]
        return pltpu.make_async_copy(src.at[r0:r1, c0:c1], dst.at[r0:r1, c0:c1], sem_in.at[n])

    def cp_xr():
        return cp_rows(x_hbm.at[0], x_v, pl.ds(R1, S - R1), s_xr)

    def cp_gw():
        return pltpu.make_async_copy(gw_hbm, gw_v, sem_in.at[s_gw])

    def cp_g(c):
        return cp_cols(wg_hbm, wg_v, _ds(c, FC), s_w + 3 * c)

    def cp_u(c):
        return cp_cols(wu_hbm, wu_v, _ds(c, FC), s_w + 3 * c + 1)

    def cp_d(c):
        return cp_rows(wd_hbm, wd_v, _ds(c, FC), s_w + 3 * c + 2)

    def cp_wq(t):
        return cp_rows(wqkv_hbm, wqkv_v, _ds(t, D // NAUX), s_q + t)

    def cp_wo(t):
        return cp_cols(wo_hbm, wo_v, _ds(t, D // NAUX), s_o + t)

    def cp_out(i):
        sl = _ds(i, MA)
        return pltpu.make_async_copy(out_v.at[sl, :], out_hbm.at[0, sl, :], sem_out.at[i])

    for n in range(len(PEEL_COPIES)):
        cp_peel(n).start()

    def issue(c, carry):
        cp_g(c).start(); cp_u(c).start(); cp_d(c).start()

        @pl.when(jnp.logical_and(c >= 2, c < 2 + NAUX))
        def _():
            cp_wq(c - 2).start(); cp_wo(c - 2).start()
        return carry

    lax.fori_loop(1, nc, issue, 0)
    cp_gw().start()
    cp_xr().start()

    lane8 = lax.broadcasted_iota(jnp.int32, (8, LANES), 1)
    odd = (lane8 & 1) == 1
    row8 = lax.broadcasted_iota(jnp.int32, (8, LANES), 0)

    def tile(m, t, r=0):
        return m[r:r + 8, t * LANES:(t + 1) * LANES]

    def after(never, tok, u32):
        return jnp.concatenate(
            [jnp.concatenate([jnp.where(never, tok, tile(u32, t, r))
                              for t in range(u32.shape[1] // LANES)], axis=1)
             for r in range(0, u32.shape[0], 8)], axis=0)

    def waits_for(never, toks, w):
        if not toks:
            return w
        w = _pk(w)
        top = [jnp.where(never, toks[t], tile(w, t)) if t in toks else tile(w, t)
               for t in range(w.shape[1] // LANES)]
        return _bf(jnp.concatenate([jnp.concatenate(top, axis=1), w[8:, :]], axis=0))

    def permute_put(slot, u32):
        for g in range(2 * H):
            tmp_v[slot, pl.ds((g // 2) * PITCH + (g % 2) * 8, 8), :] = u32[g * 8:(g + 1) * 8, :]

    def permute_get(slot, dst, col, sec, never, toks):
        for n in range(D // 16):
            je, a = divmod(n, H // 8)
            val = tmp_v[slot, pl.ds(8 * (je % 2) + je // 2 + a * 8 * PITCH, 8, stride=PITCH), :]
            dst[col, _ds(sec, D // 2, 8, n * 8, 8), :] = jnp.where(never, toks[n], val)

    def wq_put(slot, kb, sec, never, tok):
        raw = _pk(wqkv_v[_ds(kb, LANES), _ds(sec, D)])
        u32 = _pk(_bf(after(never, tok, raw)).T)
        permute_put(slot, u32)
        done = u32[56:64, :]
        for t in range(1, NCH):
            done = done | u32[t * 64 + 56:t * 64 + 64, :]
        return done

    def wo_put(slot, c, never, toks):
        n = D // len(toks)
        permute_put(slot, jnp.concatenate(
            [after(never, tok, _pk(wo_v[i * n:(i + 1) * n, _ds(c, LANES)]))
             for i, tok in enumerate(toks)], axis=0))

    def qkv(xa):
        for sec, dst, r0 in ((1, k_v, HALO), (0, q_v, 0), (2, v_v, HALO)):
            w = jnp.concatenate([wt_v[kb, sec * (D // 2):(sec + 1) * (D // 2), :] for kb in range(NCH)],
                                axis=1)
            res = _dot_nt(xa, _bf(w))
            for j in range(NCH):
                dst[j, r0:r0 + MA, :] = res[:, j * LANES:(j + 1) * LANES]

    def attn8(r, row0, never, tok, gate):
        sc = jnp.where(never, tok, scale * LOG2E)
        q = [q_v[j, r:r + 8, :] * sc for j in range(NCH)]
        logits = []
        valid = {}
        for w in range(WIN):
            lo = HALO + r - DIL * w
            s = q[0] * k_v[0, lo:lo + 8, :]
            for j in range(1, NCH):
                s = s + q[j] * k_v[j, lo:lo + 8, :]
            s = s + pltpu.roll(s, 64, 1)
            s = s + jnp.where(odd, pltpu.roll(s, 1, 1), pltpu.roll(s, LANES - 1, 1))
            if r - DIL * w < 0:
                valid[w] = row8 + (row0 + r - DIL * w) >= 0
                s = jnp.where(valid[w], s, NEG * LOG2E)
            logits.append(s)
        m = logits[0]
        for w in range(1, WIN):
            m = jnp.maximum(m, logits[w])
        p = [jnp.exp2(l - m) for l in logits]
        den = p[0]
        for w in range(1, WIN):
            den = den + p[w]
        inv = pl.reciprocal(den, approx=True)
        inv = inv * (2.0 - den * inv) * gate
        p = [pw * inv for pw in p]
        pm = None
        for w in valid:
            t = jnp.where(valid[w], 0.0, p[w])
            pm = t if pm is None else pm + t
        outs = []
        for j in range(NCH):
            acc = p[0] * v_v[j, HALO + r:HALO + r + 8, :]
            for w in range(1, WIN):
                lo = HALO + r - DIL * w
                acc = acc + p[w] * v_v[j, lo:lo + 8, :]
            if pm is not None:
                acc = acc + pm * v_v[j, HALO:HALO + 1, :]
            outs.append(acc)
        return outs, pltpu.bitcast(inv, U32)

    def attn16(r, i, never, tok_g, tok_a, tok_b):
        xg = _pk(x_v[_ds(i, MA, 16, r, 16), :])
        xg = _bf(after(never, pltpu.bitcast(tok_g, U32), xg)).astype(F32)
        z = jnp.sum(xg * gw_v[...].astype(F32).reshape(1, D), axis=-1, keepdims=True)
        th = 0.5 * jnp.tanh(jnp.broadcast_to(0.5 * z, (16, LANES)))
        gate = 0.5 + th
        og_v[r:r + 16, :] = 0.5 - th
        a, done_a = attn8(r, i * MA, never, tok_a, gate[0:8])
        b, done_b = attn8(r + 8, i * MA, never, tok_b, gate[8:16])
        for j in range(NCH):
            o_v[r // 2:r // 2 + 8, j * LANES:(j + 1) * LANES] = _pk(
                jnp.concatenate([a[j], b[j]], axis=0).astype(BF16))
        return done_a, done_b

    def clear(j, carry):
        k_v[j, MA:MA + HALO, :] = jnp.zeros((HALO, LANES), F32)
        v_v[j, MA:MA + HALO, :] = jnp.zeros((HALO, LANES), F32)
        wqkv_v[_ds(j, 16, base=D), 0:D] = jnp.zeros((16, D), BF16)
        wo_v[_ds(j, LANES), D:] = jnp.zeros((LANES, LANES), BF16)
        return carry

    lax.fori_loop(0, NCH, clear, 0)

    parts = {}

    def gather(kind, c0, c1):
        keys = sorted(k for k in parts if k[0] == kind and c0 <= k[1] < c1)
        cols = [jnp.concatenate([parts.pop(k) for k in keys if k[1] == cc], axis=0)
                for cc in sorted({k[1] for k in keys})]
        return jnp.concatenate(cols, axis=1)

    for waits, work in PEEL_STEPS:
        for n in waits:
            cp_peel(n).wait()
        for kind, r0, r1, c0, c1, k0, k1 in work:
            if kind in "gu":
                val = _dot(x_v[r0:r1, k0:k1], (wg_v if kind == "g" else wu_v)[k0:k1, c0:c1])
                parts[kind, c0, r0] = val + gather(kind, c0, c1) if k0 else val
            elif kind == "h":
                val = jnp.maximum(gather("g", c0, c1), 0.0) * gather("u", c0, c1)
                parts[kind, c0, r0] = val.astype(BF16)
            else:
                b_v[0:R1, :] = _dot(gather("h", c0, c1), wd_v[c0:c1, :])

    def p1_body(c, carry):
        aux = jnp.logical_and(c >= 2, c < 2 + NAUX)
        ta = jnp.clip(c - 2, 0, NAUX - 1)
        cp_g(c).wait(); cp_u(c).wait(); cp_d(c).wait()
        pl.when(aux)(cp_wq(ta).wait)
        pl.when(aux)(cp_wo(ta).wait)
        uq = [UQ * (c - 2) + t for t in range(UQ)]
        uo = [UO * (c - 2) + t for t in range(UO)]
        uq = [jnp.where(jnp.logical_and(u >= 0, u < NU), u, NU) for u in uq]
        uo = [jnp.where(jnp.logical_and(u >= 0, u < NCH), u, NCH) for u in uo]
        uq = [(lax.div(u, 3), lax.rem(u, 3)) for u in uq]
        xv = x_v[0:R1, :]
        never = row8 + c < 0
        res = []
        done = {}
        for m in range(2 * nt):
            w = (wg_v if m < nt else wu_v)[:, _ds(c, FC, LANES, (m % nt) * LANES, LANES)]
            r = _dot(xv, waits_for(never, done.get(m), w))
            res.append(r)
            if m < UQ:
                done[m + P1_LAG] = {0: wq_put(m, *uq[m], never, pltpu.bitcast(tile(r, 0), U32))}
            if 0 <= m - P1_LAG < UQ:
                toks = [pltpu.bitcast(tile(r, 0, rr), U32) for rr in range(0, R1, 8)]
                permute_get(m - P1_LAG, wt_v, *uq[m - P1_LAG], never, toks)
        g = jnp.concatenate(res[:nt], axis=1)
        u = jnp.concatenate(res[nt:], axis=1)
        r = _dot((jnp.maximum(g, 0.0) * u).astype(BF16), wd_v[_ds(c, FC), :])
        b_v[0:R1, :] += r
        for t in range(UO):
            toks = [pltpu.bitcast(tile(r, tt, rr), U32) for tt in WO_TILES[t] for rr in range(0, R1, R1 // 4)]
            wo_put(UQ + t, uo[t], never, toks)
            toks = [pltpu.bitcast(tile(r, WO_TILES[t][-1] + 1, rr), U32) for rr in range(0, R1, 8)]
            permute_get(UQ + t, wop_v, uo[t], 0, never, toks)
        return carry

    lax.fori_loop(1, nc, p1_body, 0)
    cp_gw().wait()
    cp_xr().wait()

    def p2_body(i, carry):
        ra = _ds(i, MA)
        rf = _ds(i, MF, base=R1, align=16)
        k_v[:, 0:HALO, :] = k_v[:, MA:MA + HALO, :]
        v_v[:, 0:HALO, :] = v_v[:, MA:MA + HALO, :]
        never = row8 + i < 0
        groups = iter(range(0, MA, 16))

        def attn_group(m, k):
            r = next(groups, None)
            if r is None:
                return None
            return dict(zip(DEADLINES[k], attn16(r, i, never, *(tile(m, t) for t in TOKS[k]))))

        dl = None
        for c in range(nc):
            cols = slice(c * FC, (c + 1) * FC)
            xv = x_v[rf, :]
            if c == 0:
                wk = wg_v[:, cols]
                g = _dot(jnp.concatenate([xv[:, t * LANES:(t + 1) * LANES] for t in K_ORDER], axis=1),
                         jnp.concatenate([wk[t * LANES:(t + 1) * LANES, :] for t in K_ORDER], axis=0))
                h = (jnp.maximum(g, 0.0) * _dot(xv, wu_v[:, cols])).astype(BF16)
                b_v[rf, :] = _dot(h, wd_v[cols, :])
                qkv(x_v[ra, :])
                continue
            g = _dot(xv, waits_for(never, dl, wg_v[:, cols]))
            dl = attn_group(g, 0)
            u = _dot(xv, waits_for(never, dl, wu_v[:, cols]))
            dl = attn_group(u, 1)
            h = (jnp.maximum(g, 0.0) * u).astype(BF16)
            r = _dot(h, waits_for(never, dl, wd_v[cols, :]))
            b_v[rf, :] += r
            dl = attn_group(r, 2)
        a = _dot(_bf(o_v[...]), _bf(jnp.concatenate([wop_v[c] for c in range(NCH)], axis=1)))
        og = jnp.concatenate([og_v[...]] * NCH, axis=1)
        out_v[ra, :] = (a + og * b_v[ra, :]).astype(BF16)
        cp_out(i).start()
        return carry

    lax.fori_loop(0, NIT, p2_body, 0)
    for i in range(NIT):
        cp_out(i).wait()


@jax.jit
def pallas_gated_mix__sliding_local_dilated__glu_gated_reglu__prompt_kernel(
    A_x: jax.Array,
    A_wqkv: jax.Array,
    A_wo: jax.Array,
    B_x: jax.Array,
    B_W_gate: jax.Array,
    B_W_up: jax.Array,
    B_W_down: jax.Array,
    gate_w: jax.Array,
):
    B, S, D = A_x.shape
    assert B == 1
    F = B_W_gate.shape[1]
    NCH = D // LANES
    MA = S // NIT
    n_in = len(PEEL_COPIES) + 2 + 3 * (F // FC - 1) + 2 * NAUX

    def kernel(*refs):
        def once(_, c):
            _kernel(*refs, S=S, D=D, F=F)
            return c

        lax.fori_loop(0, pl.program_id(0) + 1, once, 0)

    any_spec = pl.BlockSpec(memory_space=pl.ANY)
    return pl.pallas_call(
        kernel,
        grid=(1,),
        in_specs=[any_spec] * 7,
        out_specs=any_spec,
        out_shape=jax.ShapeDtypeStruct((B, S, D), A_x.dtype),
        scratch_shapes=[
            pltpu.VMEM((S, D), BF16),
            pltpu.VMEM((D + LANES, 3 * D), BF16),
            pltpu.VMEM((D, D + LANES), BF16),
            pltpu.VMEM((D, F), BF16),
            pltpu.VMEM((D, F), BF16),
            pltpu.VMEM((F, D), BF16),
            pltpu.VMEM((D,), BF16),
            pltpu.VMEM((NCH + 1, 3 * D // 2, LANES), U32),
            pltpu.VMEM((NCH + 1, D // 2, LANES), U32),
            pltpu.VMEM((UQ + UO, TMP_ROWS, LANES), U32),
            pltpu.VMEM((S, D), F32),
            pltpu.VMEM((NCH, MA, LANES), F32),
            pltpu.VMEM((NCH, HALO + MA, LANES), F32),
            pltpu.VMEM((NCH, HALO + MA, LANES), F32),
            pltpu.VMEM((MA // 2, D), U32),
            pltpu.VMEM((MA, LANES), F32),
            pltpu.VMEM((S, D), BF16),
            pltpu.SemaphoreType.DMA((n_in,)),
            pltpu.SemaphoreType.DMA((NIT,)),
        ],
        compiler_params=pltpu.CompilerParams(
            vmem_limit_bytes=100 * 1024 * 1024,
            disable_semaphore_checks=True,
            disable_bounds_checks=True,
        ),
    )(A_x, A_wqkv, A_wo, B_W_gate, B_W_up, B_W_down, gate_w)
```

```python
import jax
import jax.numpy as jnp
from jax import lax
import jax.experimental.pallas as pl
import jax.experimental.pallas.tpu as pltpu

H = 32
WIN = 8
DIL = 2
NEG = -1e9

LANES = 128
LOG2E = 1.4426950408889634
HALO = 16

R1 = 512
FC = 512
NIT = 8
UQ = 5
UO = 2
NAUX = 4
PITCH = 17
TMP_ROWS = 552

TOKS = ((0, 1, 3), (0, 1, 3), (0, 2, 6))
DEADLINES = ((0, 2), (0, 4), (0, 2))
P1_LAG = 2
WO_TILES = ((0, 1), (3, 4))
K_ORDER = (3, 2, 1, 0, 7, 6, 5, 4)

PEEL_COPIES = (("x", 0, 256, 0, 512), ("g", 0, 512, 0, 256), ("x", 256, 512, 0, 512),
               ("g", 0, 512, 256, 512), ("u", 0, 512, 0, 512), ("x", 0, 512, 512, 1024),
               ("g", 512, 1024, 0, 512), ("u", 512, 1024, 0, 256), ("u", 512, 1024, 256, 512),
               ("d", 0, 512, 0, 1024))
PEEL_STEPS = (
    ((0, 1), (("g", 0, 256, 0, 256, 0, 512),)),
    ((2,), (("g", 256, 512, 0, 256, 0, 512),)),
    ((3,), (("g", 0, 512, 256, 512, 0, 512),)),
    ((4,), (("u", 0, 512, 0, 256, 0, 512), ("u", 0, 512, 256, 512, 0, 512))),
    ((5, 6, 7), (("g", 0, 512, 0, 256, 512, 1024), ("g", 0, 512, 256, 512, 512, 1024),
                 ("u", 0, 512, 0, 256, 512, 1024), ("h", 0, 512, 0, 256, 0, 0))),
    ((8, 9), (("u", 0, 512, 256, 512, 512, 1024), ("h", 0, 512, 256, 512, 0, 0),
              ("d", 0, 512, 0, 512, 0, 0))),
)

F32 = jnp.float32
BF16 = jnp.bfloat16
U32 = jnp.uint32


def _dot(a, b):
    return jnp.dot(a, b, preferred_element_type=F32)


def _dot_nt(a, b):
    return lax.dot_general(a, b, (((1,), (1,)), ((), ())), preferred_element_type=F32)


def _pk(v):
    return pltpu.bitcast(v, U32)


def _bf(v):
    return pltpu.bitcast(v, BF16)


def _ds(i, step, size=None, base=0, align=None):
    size = step if size is None else size
    start = base + i * step
    if not isinstance(start, int):
        start = pl.multiple_of(start, step if align is None else align)
    return pl.ds(start, size)


def _kernel(x_hbm, wqkv_hbm, wo_hbm, wg_hbm, wu_hbm, wd_hbm, gw_hbm, out_hbm,
            x_v, wqkv_v, wo_v, wg_v, wu_v, wd_v, gw_v,
            wt_v, wop_v, tmp_v, b_v, q_v, k_v, v_v, o_v, og_v, out_v,
            sem_in, sem_out, *, S, D, F):
    NCH = D // LANES
    scale = (D // H) ** -0.5
    nc = F // FC
    nt = FC // LANES
    MF = (S - R1) // NIT
    MA = S // NIT
    NU = 3 * NCH
    assert UQ * (nc - 2) >= NU and UO * (nc - 2) >= NCH and MA // 16 <= 3 * (nc - 1)

    s_gw = len(PEEL_COPIES)
    s_xr = s_gw + 1
    s_w = s_xr + 1 - 3
    s_q = s_w + 3 * nc
    s_o = s_q + NAUX

    def cp_rows(src, dst, sl, s):
        return pltpu.make_async_copy(src.at[sl, :], dst.at[sl, :], sem_in.at[s])

    def cp_cols(src, dst, sl, s):
        return pltpu.make_async_copy(src.at[:, sl], dst.at[:, sl], sem_in.at[s])

    def cp_peel(n):
        kind, r0, r1, c0, c1 = PEEL_COPIES[n]
        src, dst = {"x": (x_hbm.at[0], x_v), "g": (wg_hbm, wg_v), "u": (wu_hbm, wu_v), "d": (wd_hbm, wd_v)}[kind]
        return pltpu.make_async_copy(src.at[r0:r1, c0:c1], dst.at[r0:r1, c0:c1], sem_in.at[n])

    def cp_xr():
        return cp_rows(x_hbm.at[0], x_v, pl.ds(R1, S - R1), s_xr)

    def cp_gw():
        return pltpu.make_async_copy(gw_hbm, gw_v, sem_in.at[s_gw])

    def cp_g(c):
        return cp_cols(wg_hbm, wg_v, _ds(c, FC), s_w + 3 * c)

    def cp_u(c):
        return cp_cols(wu_hbm, wu_v, _ds(c, FC), s_w + 3 * c + 1)

    def cp_d(c):
        return cp_rows(wd_hbm, wd_v, _ds(c, FC), s_w + 3 * c + 2)

    def cp_wq(t):
        return cp_rows(wqkv_hbm, wqkv_v, _ds(t, D // NAUX), s_q + t)

    def cp_wo(t):
        return cp_cols(wo_hbm, wo_v, _ds(t, D // NAUX), s_o + t)

    def cp_out(i):
        sl = _ds(i, MA)
        return pltpu.make_async_copy(out_v.at[sl, :], out_hbm.at[0, sl, :], sem_out.at[i])

    for n in range(len(PEEL_COPIES)):
        cp_peel(n).start()

    def issue(c, carry):
        cp_g(c).start(); cp_u(c).start(); cp_d(c).start()

        @pl.when(jnp.logical_and(c >= 2, c < 2 + NAUX))
        def _():
            cp_wq(c - 2).start(); cp_wo(c - 2).start()
        return carry

    lax.fori_loop(1, nc, issue, 0)
    cp_gw().start()
    cp_xr().start()

    lane8 = lax.broadcasted_iota(jnp.int32, (8, LANES), 1)
    odd = (lane8 & 1) == 1
    row8 = lax.broadcasted_iota(jnp.int32, (8, LANES), 0)

    def tile(m, t, r=0):
        return m[r:r + 8, t * LANES:(t + 1) * LANES]

    def after(never, tok, u32):
        return jnp.concatenate(
            [jnp.concatenate([jnp.where(never, tok, tile(u32, t, r))
                              for t in range(u32.shape[1] // LANES)], axis=1)
             for r in range(0, u32.shape[0], 8)], axis=0)

    def waits_for(never, toks, w):
        if not toks:
            return w
        w = _pk(w)
        top = [jnp.where(never, toks[t], tile(w, t)) if t in toks else tile(w, t)
               for t in range(w.shape[1] // LANES)]
        return _bf(jnp.concatenate([jnp.concatenate(top, axis=1), w[8:, :]], axis=0))

    def permute_put(slot, u32):
        for g in range(2 * H):
            tmp_v[slot, pl.ds((g // 2) * PITCH + (g % 2) * 8, 8), :] = u32[g * 8:(g + 1) * 8, :]

    def permute_get(slot, dst, col, sec, never, toks):
        for n in range(D // 16):
            je, a = divmod(n, H // 8)
            val = tmp_v[slot, pl.ds(8 * (je % 2) + je // 2 + a * 8 * PITCH, 8, stride=PITCH), :]
            dst[col, _ds(sec, D // 2, 8, n * 8, 8), :] = jnp.where(never, toks[n], val)

    def wq_put(slot, kb, sec, never, tok):
        raw = _pk(wqkv_v[_ds(kb, LANES), _ds(sec, D)])
        u32 = _pk(_bf(after(never, tok, raw)).T)
        permute_put(slot, u32)
        done = u32[56:64, :]
        for t in range(1, NCH):
            done = done | u32[t * 64 + 56:t * 64 + 64, :]
        return done

    def wo_put(slot, c, never, toks):
        n = D // len(toks)
        permute_put(slot, jnp.concatenate(
            [after(never, tok, _pk(wo_v[i * n:(i + 1) * n, _ds(c, LANES)]))
             for i, tok in enumerate(toks)], axis=0))

    def qkv(xa):
        for sec, dst, r0 in ((1, k_v, HALO), (0, q_v, 0), (2, v_v, HALO)):
            w = jnp.concatenate([wt_v[kb, sec * (D // 2):(sec + 1) * (D // 2), :] for kb in range(NCH)],
                                axis=1)
            res = _dot_nt(xa, _bf(w))
            for j in range(NCH):
                dst[j, r0:r0 + MA, :] = res[:, j * LANES:(j + 1) * LANES]

    def attn8(r, row0, never, tok, gate):
        sc = jnp.where(never, tok, scale * LOG2E)
        q = [q_v[j, r:r + 8, :] * sc for j in range(NCH)]
        logits = []
        valid = {}
        for w in range(WIN):
            lo = HALO + r - DIL * w
            s = q[0] * k_v[0, lo:lo + 8, :]
            for j in range(1, NCH):
                s = s + q[j] * k_v[j, lo:lo + 8, :]
            s = s + pltpu.roll(s, 64, 1)
            s = s + jnp.where(odd, pltpu.roll(s, 1, 1), pltpu.roll(s, LANES - 1, 1))
            if r - DIL * w < 0:
                valid[w] = row8 + (row0 + r - DIL * w) >= 0
                s = jnp.where(valid[w], s, NEG * LOG2E)
            logits.append(s)
        m = logits[0]
        for w in range(1, WIN):
            m = jnp.maximum(m, logits[w])
        p = [jnp.exp2(l - m) for l in logits]
        den = p[0]
        for w in range(1, WIN):
            den = den + p[w]
        inv = pl.reciprocal(den, approx=True)
        inv = inv * (2.0 - den * inv) * gate
        p = [pw * inv for pw in p]
        pm = None
        for w in valid:
            t = jnp.where(valid[w], 0.0, p[w])
            pm = t if pm is None else pm + t
        outs = []
        for j in range(NCH):
            acc = p[0] * v_v[j, HALO + r:HALO + r + 8, :]
            for w in range(1, WIN):
                lo = HALO + r - DIL * w
                acc = acc + p[w] * v_v[j, lo:lo + 8, :]
            if pm is not None:
                acc = acc + pm * v_v[j, HALO:HALO + 1, :]
            outs.append(acc)
        return outs, pltpu.bitcast(inv, U32)

    def attn16(r, i, never, tok_g, tok_a, tok_b):
        xg = _pk(x_v[_ds(i, MA, 16, r, 16), :])
        xg = _bf(after(never, pltpu.bitcast(tok_g, U32), xg)).astype(F32)
        z = jnp.sum(xg * gw_v[...].astype(F32).reshape(1, D), axis=-1, keepdims=True)
        th = 0.5 * jnp.tanh(jnp.broadcast_to(0.5 * z, (16, LANES)))
        gate = 0.5 + th
        og_v[r:r + 16, :] = 0.5 - th
        a, done_a = attn8(r, i * MA, never, tok_a, gate[0:8])
        b, done_b = attn8(r + 8, i * MA, never, tok_b, gate[8:16])
        for j in range(NCH):
            o_v[r // 2:r // 2 + 8, j * LANES:(j + 1) * LANES] = _pk(
                jnp.concatenate([a[j], b[j]], axis=0).astype(BF16))
        return done_a, done_b

    def clear(j, carry):
        k_v[j, MA:MA + HALO, :] = jnp.zeros((HALO, LANES), F32)
        v_v[j, MA:MA + HALO, :] = jnp.zeros((HALO, LANES), F32)
        wqkv_v[_ds(j, 16, base=D), 0:D] = jnp.zeros((16, D), BF16)
        wo_v[_ds(j, LANES), D:] = jnp.zeros((LANES, LANES), BF16)
        return carry

    lax.fori_loop(0, NCH, clear, 0)

    parts = {}

    def gather(kind, c0, c1):
        keys = sorted(k for k in parts if k[0] == kind and c0 <= k[1] < c1)
        cols = [jnp.concatenate([parts.pop(k) for k in keys if k[1] == cc], axis=0)
                for cc in sorted({k[1] for k in keys})]
        return jnp.concatenate(cols, axis=1)

    for waits, work in PEEL_STEPS:
        for n in waits:
            cp_peel(n).wait()
        for kind, r0, r1, c0, c1, k0, k1 in work:
            if kind in "gu":
                val = _dot(x_v[r0:r1, k0:k1], (wg_v if kind == "g" else wu_v)[k0:k1, c0:c1])
                parts[kind, c0, r0] = val + gather(kind, c0, c1) if k0 else val
            elif kind == "h":
                val = jnp.maximum(gather("g", c0, c1), 0.0) * gather("u", c0, c1)
                parts[kind, c0, r0] = val.astype(BF16)
            else:
                b_v[0:R1, :] = _dot(gather("h", c0, c1), wd_v[c0:c1, :])

    def p1_body(c, carry):
        aux = jnp.logical_and(c >= 2, c < 2 + NAUX)
        ta = jnp.clip(c - 2, 0, NAUX - 1)
        cp_g(c).wait(); cp_u(c).wait(); cp_d(c).wait()
        pl.when(aux)(cp_wq(ta).wait)
        pl.when(aux)(cp_wo(ta).wait)
        uq = [UQ * (c - 2) + t for t in range(UQ)]
        uo = [UO * (c - 2) + t for t in range(UO)]
        uq = [jnp.where(jnp.logical_and(u >= 0, u < NU), u, NU) for u in uq]
        uo = [jnp.where(jnp.logical_and(u >= 0, u < NCH), u, NCH) for u in uo]
        uq = [(lax.div(u, 3), lax.rem(u, 3)) for u in uq]
        xv = x_v[0:R1, :]
        never = row8 + c < 0
        res = []
        done = {}
        for m in range(2 * nt):
            w = (wg_v if m < nt else wu_v)[:, _ds(c, FC, LANES, (m % nt) * LANES, LANES)]
            r = _dot(xv, waits_for(never, done.get(m), w))
            res.append(r)
            if m < UQ:
                done[m + P1_LAG] = {0: wq_put(m, *uq[m], never, pltpu.bitcast(tile(r, 0), U32))}
            if 0 <= m - P1_LAG < UQ:
                toks = [pltpu.bitcast(tile(r, 0, rr), U32) for rr in range(0, R1, 8)]
                permute_get(m - P1_LAG, wt_v, *uq[m - P1_LAG], never, toks)
        g = jnp.concatenate(res[:nt], axis=1)
        u = jnp.concatenate(res[nt:], axis=1)
        r = _dot((jnp.maximum(g, 0.0) * u).astype(BF16), wd_v[_ds(c, FC), :])
        b_v[0:R1, :] += r
        for t in range(UO):
            toks = [pltpu.bitcast(tile(r, tt, rr), U32) for tt in WO_TILES[t] for rr in range(0, R1, R1 // 4)]
            wo_put(UQ + t, uo[t], never, toks)
            toks = [pltpu.bitcast(tile(r, WO_TILES[t][-1] + 1, rr), U32) for rr in range(0, R1, 8)]
            permute_get(UQ + t, wop_v, uo[t], 0, never, toks)
        return carry

    lax.fori_loop(1, nc, p1_body, 0)
    cp_gw().wait()
    cp_xr().wait()

    def p2_body(i, carry):
        ra = _ds(i, MA)
        rf = _ds(i, MF, base=R1, align=16)
        k_v[:, 0:HALO, :] = k_v[:, MA:MA + HALO, :]
        v_v[:, 0:HALO, :] = v_v[:, MA:MA + HALO, :]
        never = row8 + i < 0
        groups = iter(range(0, MA, 16))

        def attn_group(m, k):
            r = next(groups, None)
            if r is None:
                return None
            return dict(zip(DEADLINES[k], attn16(r, i, never, *(tile(m, t) for t in TOKS[k]))))

        dl = None
        for c in range(nc):
            cols = slice(c * FC, (c + 1) * FC)
            xv = x_v[rf, :]
            if c == 0:
                wk = wg_v[:, cols]
                g = _dot(jnp.concatenate([xv[:, t * LANES:(t + 1) * LANES] for t in K_ORDER], axis=1),
                         jnp.concatenate([wk[t * LANES:(t + 1) * LANES, :] for t in K_ORDER], axis=0))
                h = (jnp.maximum(g, 0.0) * _dot(xv, wu_v[:, cols])).astype(BF16)
                b_v[rf, :] = _dot(h, wd_v[cols, :])
                qkv(x_v[ra, :])
                continue
            g = _dot(xv, waits_for(never, dl, wg_v[:, cols]))
            dl = attn_group(g, 0)
            u = _dot(xv, waits_for(never, dl, wu_v[:, cols]))
            dl = attn_group(u, 1)
            h = (jnp.maximum(g, 0.0) * u).astype(BF16)
            r = _dot(h, waits_for(never, dl, wd_v[cols, :]))
            b_v[rf, :] += r
            dl = attn_group(r, 2)
        a = _dot(_bf(o_v[...]), _bf(jnp.concatenate([wop_v[c] for c in range(NCH)], axis=1)))
        og = jnp.concatenate([og_v[...]] * NCH, axis=1)
        out_v[ra, :] = (a + og * b_v[ra, :]).astype(BF16)
        cp_out(i).start()
        return carry

    lax.fori_loop(0, NIT, p2_body, 0)
    for i in range(NIT):
        cp_out(i).wait()


@jax.jit
def pallas_gated_mix__sliding_local_dilated__glu_gated_reglu__prompt_kernel(
    A_x: jax.Array,
    A_wqkv: jax.Array,
    A_wo: jax.Array,
    B_x: jax.Array,
    B_W_gate: jax.Array,
    B_W_up: jax.Array,
    B_W_down: jax.Array,
    gate_w: jax.Array,
):
    B, S, D = A_x.shape
    assert B == 1
    F = B_W_gate.shape[1]
    NCH = D // LANES
    MA = S // NIT
    n_in = len(PEEL_COPIES) + 2 + 3 * (F // FC - 1) + 2 * NAUX

    def kernel(*refs):
        def once(_, c):
            _kernel(*refs, S=S, D=D, F=F)
            return c

        lax.fori_loop(0, pl.program_id(0) + 1, once, 0)

    any_spec = pl.BlockSpec(memory_space=pl.ANY)
    return pl.pallas_call(
        kernel,
        grid=(1,),
        in_specs=[any_spec] * 7,
        out_specs=any_spec,
        out_shape=jax.ShapeDtypeStruct((B, S, D), A_x.dtype),
        scratch_shapes=[
            pltpu.VMEM((S, D), BF16),
            pltpu.VMEM((D + LANES, 3 * D), BF16),
            pltpu.VMEM((D, D + LANES), BF16),
            pltpu.VMEM((D, F), BF16),
            pltpu.VMEM((D, F), BF16),
            pltpu.VMEM((F, D), BF16),
            pltpu.VMEM((D,), BF16),
            pltpu.VMEM((NCH + 1, 3 * D // 2, LANES), U32),
            pltpu.VMEM((NCH + 1, D // 2, LANES), U32),
            pltpu.VMEM((UQ + UO, TMP_ROWS, LANES), U32),
            pltpu.VMEM((S, D), F32),
            pltpu.VMEM((NCH, MA, LANES), F32),
            pltpu.VMEM((NCH, HALO + MA, LANES), F32),
            pltpu.VMEM((NCH, HALO + MA, LANES), F32),
            pltpu.VMEM((MA // 2, D), U32),
            pltpu.VMEM((MA, LANES), F32),
            pltpu.VMEM((S, D), BF16),
            pltpu.SemaphoreType.DMA((n_in,)),
            pltpu.SemaphoreType.DMA((NIT,)),
        ],
        compiler_params=pltpu.CompilerParams(
            vmem_limit_bytes=100 * 1024 * 1024,
            disable_semaphore_checks=True,
            disable_bounds_checks=True,
        ),
    )(A_x, A_wqkv, A_wo, B_W_gate, B_W_up, B_W_down, gate_w)
```
